```python
import jax
import jax.numpy as jnp

def _softmax(x, axis=-1):
    return jax.nn.softmax(x, axis=axis)

def _gelu(x):
    return jax.nn.gelu(x, approximate=True)

def _silu(x):
    return jax.nn.silu(x)

def _sigmoid(x):
    return jax.nn.sigmoid(x)

def _layernorm(x, axis=-1, eps=1e-05):
    m = jnp.mean(x, axis=axis, keepdims=True)
    v = jnp.var(x, axis=axis, keepdims=True)
    return (x - m) / jnp.sqrt(v + eps)

def _scatter_add(tgt, idx, src, axis=0):
    return tgt.at[idx].add(src)

def _segment_sum(src, seg, n):
    return jax.ops.segment_sum(src, seg, n)

class _Rng:

    def __init__(self, key):
        self._k = key

    def _next(self):
        self._k, sub = jax.random.split(self._k)
        return sub

    def normal(self, shape):
        return jax.random.normal(self._next(), shape, dtype=jnp.bfloat16)

    def randint(self, lo, hi, shape):
        return jax.random.randint(self._next(), shape, lo, hi, dtype=jnp.int32)

    def uniform(self, shape, lo=0.0, hi=1.0):
        return jax.random.uniform(self._next(), shape, jnp.bfloat16, lo, hi)

    def permutation(self, n):
        return jax.random.permutation(self._next(), n)
kernel_name = 'concat_heads__memory_aug_recurrent_mem_tr__compressed_kv_cla__prompt'

def setup_inputs():
    _rng = _Rng(jax.random.key(int.from_bytes(__import__("os").urandom(4), "little")))
    _w = lambda a: (lambda t: t.astype(jnp.bfloat16) if jnp.issubdtype(t.dtype, jnp.floating) else t)(jnp.asarray(a))

    def _A_setup():
        B, S, Dm = (1, 2048, 448)
        H, Dh = (16, 256)
        M, seg = (8, 32)
        seg = min(seg, S)
        S = S // seg * seg
        return {'x': _w((lambda *s: _rng.normal(s) * 0.05)(B, S, Dm)), 'mem0': _w((lambda *s: _rng.normal(s) * 0.05)(B, M, Dm)), 'Wq': _w((lambda *s: _rng.normal(s) * 0.05)(Dm, H, Dh) * Dm ** (-0.5)), 'Wk': _w((lambda *s: _rng.normal(s) * 0.05)(Dm, H, Dh) * Dm ** (-0.5)), 'Wv': _w((lambda *s: _rng.normal(s) * 0.05)(Dm, H, Dh) * Dm ** (-0.5)), 'Wo': _w((lambda *s: _rng.normal(s) * 0.05)(H, Dh, Dm) * (H * Dh) ** (-0.5)), 'seg_len': seg}
    _A_in = _A_setup()

    def _B_setup():
        B, H, Sq, Sk, D, M = (1, 16, 2048, 2048, 256, 448)
        Dc = 4 * D
        return {'x': _w((lambda *s: _rng.normal(s) * 0.05)(B, Sq, M)), 'c_kv': _w((lambda *s: _rng.normal(s) * 0.05)(B, Sk, Dc)), 'w_q': _w((lambda *s: _rng.normal(s) * 0.05)(M, H, D) * M ** (-0.5)), 'w_uk': _w((lambda *s: _rng.normal(s) * 0.05)(Dc, H, D) * Dc ** (-0.5)), 'w_uv': _w((lambda *s: _rng.normal(s) * 0.05)(Dc, H, D) * Dc ** (-0.5)), 'w_o': _w((lambda *s: _rng.normal(s) * 0.05)(H, D, M) * (H * D) ** (-0.5))}
    _B_in = _B_setup()
    return {'A_x': _A_in['x'], 'A_mem0': _A_in['mem0'], 'A_Wq': _A_in['Wq'], 'A_Wk': _A_in['Wk'], 'A_Wv': _A_in['Wv'], 'A_Wo': _A_in['Wo'], 'A_seg_len': _A_in['seg_len'], 'B_x': _B_in['x'], 'B_c_kv': _B_in['c_kv'], 'B_w_q': _B_in['w_q'], 'B_w_uk': _B_in['w_uk'], 'B_w_uv': _B_in['w_uv'], 'B_w_o': _B_in['w_o']}

def reference(A_x, A_mem0, A_Wq, A_Wk, A_Wv, A_Wo, A_seg_len, B_x, B_c_kv, B_w_q, B_w_uk, B_w_uv, B_w_o):

    def _A_ref(x, mem0, Wq, Wk, Wv, Wo, seg_len):
        B, S, Dm = x.shape
        H, Dh = (Wq.shape[1], Wq.shape[2])
        M = mem0.shape[1]
        scale = Dh ** (-0.5)
        n_seg = S // seg_len
        L = M + seg_len
        idx = jnp.arange(L)
        mask = (idx[:, None] < M) | (idx[:, None] >= idx[None, :])
        mem = mem0
        outs = []
        for s in range(n_seg):
            xs = x[:, s * seg_len:(s + 1) * seg_len, :].copy()
            h = jnp.concatenate([mem, xs], axis=1)
            q = jnp.einsum('btd,dhe->bhte', h, Wq)
            k = jnp.einsum('btd,dhe->bhte', h, Wk)
            v = jnp.einsum('btd,dhe->bhte', h, Wv)
            scores = jnp.einsum('bhqe,bhke->bhqk', q, k) * scale
            scores = jnp.where(mask[None, None], scores, -1000000000.0)
            p = _softmax(scores, axis=-1)
            o = jnp.einsum('bhqk,bhke->bhqe', p, v)
            o = jnp.einsum('bhte,hed->btd', o, Wo)
            mem = o[:, :M, :].copy()
            outs.append(o[:, M:, :])
        return jnp.concatenate(outs, axis=1)

    def _B_ref(x, c_kv, w_q, w_uk, w_uv, w_o):
        B, Sq, M = (x.shape[0], x.shape[1], x.shape[2])
        Sk = c_kv.shape[1]
        H, D = (w_q.shape[1], w_q.shape[2])
        q = jnp.einsum('bqm,mhd->bhqd', x, w_q)
        k = jnp.einsum('bkc,chd->bhkd', c_kv, w_uk)
        v = jnp.einsum('bkc,chd->bhkd', c_kv, w_uv)
        scores = jnp.einsum('bhqd,bhkd->bhqk', q, k) * D ** (-0.5)
        off = Sk - Sq
        qi = jnp.arange(Sq)[:, None]
        kj = jnp.arange(Sk)[None, :]
        cmask = kj <= qi + off
        scores = jnp.where(cmask[None, None], scores, -1000000000.0)
        p = _softmax(scores, axis=-1)
        ctx = jnp.einsum('bhqk,bhkd->bhqd', p, v)
        return jnp.einsum('bhqd,hdm->bqm', ctx, w_o)
    a = _A_ref(A_x, A_mem0, A_Wq, A_Wk, A_Wv, A_Wo, A_seg_len)
    b = _B_ref(B_x, B_c_kv, B_w_q, B_w_uk, B_w_uv, B_w_o)
    return jnp.concatenate([a, b], axis=-1)
```

```python
import functools

import jax
import jax.numpy as jnp
from jax import lax
import jax.experimental.pallas as pl
import jax.experimental.pallas.tpu as pltpu

F32 = jnp.float32
BF16 = jnp.bfloat16
U32 = jnp.uint32
LOG2E = 1.4426950408889634
NEG = -1000000000.0
LANE = 128
NT = (((1,), (1,)), ((), ()))


def _dot(a, b):
    return jnp.dot(a, b, preferred_element_type=F32)


def _split_heads(raw, dst, i, rows, chunk, H):
    u = raw.bitcast(U32)
    pairs = H // 2
    d0 = pl.multiple_of(i * chunk, chunk)
    for c in range(raw.shape[0] // (rows * H)):
        blk = u.at[pl.ds(pl.multiple_of((c * rows + d0) * pairs, chunk * pairs), chunk * pairs)]
        for j in range(pairs):
            w = blk[pl.ds(j, chunk, stride=pairs), :]
            dst(2 * j, c)[pl.ds(d0, chunk), :] = pltpu.bitcast(w << 16, F32).astype(BF16)
            dst(2 * j + 1, c)[pl.ds(d0, chunk), :] = pltpu.bitcast(
                w & jnp.uint32(0xFFFF0000), F32).astype(BF16)


def _kernel(
    ax_hbm, mem_hbm, awq_hbm, awk_hbm, awv_hbm, awo_hbm,
    bx_hbm, ckv_hbm, bwq_hbm, buk_hbm, buv_hbm, bwo_hbm,
    out_hbm,
    q_all, out_v, ckv_v, bwo_v, bkv_p, sems, osems,
    *, S, Dm, H, D, M, seg, Dc,
):
    V = pltpu.VMEM
    DP = pl.cdiv(Dm, LANE) * LANE
    NP = DP // LANE
    HP = D // LANE
    CH = 64
    qscale = (D ** -0.5) * LOG2E

    def cp(src, dst, i):
        return pltpu.make_async_copy(src, dst, sems.at[i])

    def cpw(src, dst, i):
        return [cp(src.at[:, pl.ds(c * LANE, LANE)], dst.at[pl.ds(c * src.shape[0], src.shape[0])], i + c)
                for c in range(HP)]

    g3 = [cp(ckv_hbm, ckv_v, 12), cp(bwo_hbm, bwo_v, 17)]

    def phase1(wqkv, wo_p, xpad, mem_v, bx_v, bwq_v, bwq_p, ax_v, awq_v, awk_v, awv_v, awo_v):
        g1 = [cp(bx_hbm, bx_v, 0), *cpw(bwq_hbm, bwq_v, 1)]
        g2 = [cp(ax_hbm, ax_v, 3), cp(mem_hbm, mem_v, 4), *cpw(awq_hbm, awq_v, 5),
              *cpw(awk_hbm, awk_v, 7), *cpw(awv_hbm, awv_v, 9), cp(awo_hbm, awo_v, 11)]
        for c in g1:
            c.start()
        for c in g1:
            c.wait()
        for c in g2:
            c.start()
        RQ = 512

        def wq_prep(i, carry):
            _split_heads(bwq_v, lambda h, c: bwq_p.at[h * HP + c], i, Dm, CH, H)
            return carry

        lax.fori_loop(0, Dm // CH, wq_prep, 0)

        def q_body(h, carry):
            w = jnp.concatenate([bwq_p[h * HP + c] for c in range(HP)], axis=1)
            for r in range(S // RQ):
                q = _dot(bx_v[r * RQ:(r + 1) * RQ, :], w)
                q_all[h, r * RQ:(r + 1) * RQ, :] = (q * qscale).astype(BF16)
            return carry

        lax.fori_loop(0, H, q_body, 0)
        for c in g3:
            c.start()
        for c in g2:
            c.wait()

        def wqkv_prep(i, carry):
            for t, raw in enumerate((awq_v, awk_v, awv_v)):
                _split_heads(raw, lambda h, c: wqkv.at[(h * 3 + t) * HP + c], i, Dm, CH, H)
            return carry

        lax.fori_loop(0, Dm // CH, wqkv_prep, 0)

        def prep_body(h, carry):
            for p in range(3 * HP):
                wqkv[h * 3 * HP + p, Dm:DP, :] = jnp.zeros((DP - Dm, LANE), BF16)
            r0 = pl.multiple_of(h * D, D)
            wo = awo_v[pl.ds(r0, D), :]
            wo = jnp.concatenate([wo, jnp.zeros((D, DP - Dm), BF16)], axis=1)
            for c in range(NP):
                wo_p[c, pl.ds(r0, D), :] = wo[:, c * LANE:(c + 1) * LANE]
            RX = S // H
            x0 = pl.multiple_of(h * RX, RX)
            xs = ax_v[pl.ds(x0, RX), :].astype(F32)
            xpad[pl.ds(x0, RX), :] = jnp.concatenate([xs, jnp.zeros((RX, DP - Dm), F32)], axis=1)
            return carry

        lax.fori_loop(0, H, prep_body, 0)

    def phase2(wqkv, wo_p, xpad, mem_v, buk_v, buv_v):
        g4 = [*cpw(buk_hbm, buk_v, 13), *cpw(buv_hbm, buv_v, 15)]
        for c in g4:
            c.start()
        L = M + seg
        G = 2

        def a_step(s, mem):
            x0 = pl.multiple_of(s * seg, seg)
            h = jnp.concatenate([mem, xpad[pl.ds(x0, seg), :]], axis=0)
            row = lax.broadcasted_iota(jnp.int32, (L, L), 0)
            col = lax.broadcasted_iota(jnp.int32, (L, L), 1)
            mask = (row < M) | (row >= col)

            def qkv(hd):
                out = []
                for t in range(3):
                    p = (hd * 3 + t) * HP
                    out.append(jnp.concatenate([_dot(h, wqkv[p + c]) for c in range(HP)], axis=1))
                q, k, v = out
                q = (q * qscale).astype(BF16).astype(F32)
                return q, k.astype(BF16), v.astype(BF16)

            def attn(q, k, v):
                sc = lax.dot_general(q, k, NT, preferred_element_type=F32)
                sc = jnp.where(mask, sc, NEG)
                e = jnp.exp2(sc - jnp.max(sc, axis=1, keepdims=True))
                p = e * (1.0 / jnp.sum(e, axis=1, keepdims=True))
                o = _dot(p.astype(BF16).astype(F32), v)
                return o.astype(BF16).astype(F32)

            acc = [None] * NP

            def outp(g, os_):
                o = jnp.concatenate(os_, axis=1)
                for c in range(NP):
                    y = _dot(o, wo_p[c, g * G * D:(g + 1) * G * D, :])
                    acc[c] = y if acc[c] is None else acc[c] + y

            ng = H // G
            pend_qkv = None
            outs = []
            for g in range(ng):
                cur = [qkv(g * G + i) for i in range(G)]
                if pend_qkv is not None:
                    outs.append([attn(*t) for t in pend_qkv])
                pend_qkv = cur
            outp(0, outs[0])
            outs.append([attn(*t) for t in pend_qkv])
            for g in range(1, ng):
                outp(g, outs[g])
            o = jnp.concatenate(acc, axis=1).astype(BF16).astype(F32)
            out_v[pl.ds(x0, seg), 0:Dm] = o[M:, 0:Dm].astype(BF16)
            return o[:M, :]

        mem0 = jnp.concatenate([mem_v[...].astype(F32), jnp.zeros((M, DP - Dm), F32)], axis=1)
        lax.fori_loop(0, S // seg, a_step, mem0)
        for c in g4:
            c.wait()

        def wkv_prep(i, carry):
            for t, raw in enumerate((buk_v, buv_v)):
                _split_heads(raw, lambda h, c: bkv_p.at[(h * 2 + t) * HP + c], i, Dc, CH, H)
            return carry

        lax.fori_loop(0, Dc // CH, wkv_prep, 0)

    def phase12(wqkv, wo_p, xpad, mem_v):
        pl.run_scoped(
            functools.partial(phase1, wqkv, wo_p, xpad, mem_v),
            V((S, Dm), BF16), V((HP * Dm * H, LANE), BF16), V((H * HP, Dm, LANE), BF16),
            V((S, Dm), BF16), V((HP * Dm * H, LANE), BF16), V((HP * Dm * H, LANE), BF16),
            V((HP * Dm * H, LANE), BF16), V((H * D, Dm), BF16))
        pl.run_scoped(
            functools.partial(phase2, wqkv, wo_p, xpad, mem_v),
            V((HP * Dc * H, LANE), BF16), V((HP * Dc * H, LANE), BF16))

    pl.run_scoped(phase12, V((3 * H * HP, DP, LANE), BF16), V((NP, H * D, LANE), BF16),
                  V((S, DP), F32), V((M, Dm), BF16))

    def phase3(kv_v):
        for c in g3:
            c.wait()
        RK = 512
        BQ = 256

        def kv_proj(h, slot):
            w = jnp.concatenate([bkv_p[h * 2 * HP + c] for c in range(2 * HP)], axis=1)
            for r in range(S // RK):
                kv = _dot(ckv_v[r * RK:(r + 1) * RK, :], w)
                kv_v[slot, r * RK:(r + 1) * RK, :] = kv.astype(BF16)

        def attend(h, slot):
            r = lax.broadcasted_iota(jnp.int32, (BQ, BQ), 0)
            cc = lax.broadcasted_iota(jnp.int32, (BQ, BQ), 1)
            for i in range(S // BQ):
                kl = (i + 1) * BQ
                q = q_all[h, i * BQ:kl, :]
                s = lax.dot_general(q, kv_v[slot, 0:kl, 0:D], NT, preferred_element_type=F32)
                sd = jnp.where(cc <= r, s[:, kl - BQ:], NEG)
                s = jnp.concatenate([s[:, :kl - BQ], sd], axis=1) if i else sd
                p = jnp.exp2(s - jnp.max(s, axis=1, keepdims=True))
                l = jnp.sum(p, axis=1, keepdims=True)
                acc = _dot(p.astype(BF16), kv_v[slot, 0:kl, D:2 * D])
                q_all[h, i * BQ:kl, :] = (acc * (1.0 / l)).astype(BF16)

        kv_proj(0, 0)

        def b_body(h, carry):
            attend(h, h % 2)
            kv_proj(h + 1, (h + 1) % 2)
            return carry

        lax.fori_loop(0, H - 1, b_body, 0)
        attend(H - 1, (H - 1) % 2)

        RO = 256
        nro = S // RO

        def ocp(r):
            return pltpu.make_async_copy(out_v.at[pl.ds(r * RO, RO)], out_hbm.at[pl.ds(r * RO, RO)],
                                         osems.at[r])

        for r in range(nro):
            ctx = jnp.concatenate([q_all[hh, r * RO:(r + 1) * RO, :] for hh in range(H)], axis=1)
            out_v[r * RO:(r + 1) * RO, Dm:2 * Dm] = _dot(ctx, bwo_v[...]).astype(BF16)
            ocp(r).start()
        for r in range(nro):
            ocp(r).wait()

    pl.run_scoped(phase3, V((2, S, 2 * D), BF16))


@functools.partial(jax.jit, static_argnames=("A_seg_len",))
def pallas_concat_heads__memory_aug_recurrent_mem_tr__compressed_kv_cla__prompt_kernel(
    A_x, A_mem0, A_Wq, A_Wk, A_Wv, A_Wo, A_seg_len, B_x, B_c_kv, B_w_q, B_w_uk, B_w_uv, B_w_o,
):
    _, S, Dm = A_x.shape
    M = A_mem0.shape[1]
    _, H, D = A_Wq.shape
    Dc = B_c_kv.shape[2]
    seg = int(A_seg_len)
    args = (
        A_x.reshape(S, Dm), A_mem0.reshape(M, Dm),
        A_Wq.reshape(Dm * H, D), A_Wk.reshape(Dm * H, D), A_Wv.reshape(Dm * H, D),
        A_Wo.reshape(H * D, Dm),
        B_x.reshape(S, Dm), B_c_kv.reshape(S, Dc),
        B_w_q.reshape(Dm * H, D), B_w_uk.reshape(Dc * H, D), B_w_uv.reshape(Dc * H, D),
        B_w_o.reshape(H * D, Dm),
    )
    V = pltpu.VMEM
    scratch = [
        V((H, S, D), BF16), V((S, 2 * Dm), BF16), V((S, Dc), BF16), V((H * D, Dm), BF16),
        V((2 * H * D // LANE, Dc, LANE), BF16),
        pltpu.SemaphoreType.DMA((18,)), pltpu.SemaphoreType.DMA((8,)),
    ]
    out = pl.pallas_call(
        functools.partial(_kernel, S=S, Dm=Dm, H=H, D=D, M=M, seg=seg, Dc=Dc),
        out_shape=jax.ShapeDtypeStruct((S, 2 * Dm), BF16),
        in_specs=[pl.BlockSpec(memory_space=pl.ANY)] * 12,
        out_specs=pl.BlockSpec(memory_space=pl.ANY),
        scratch_shapes=scratch,
        compiler_params=pltpu.CompilerParams(vmem_limit_bytes=120 * 2**20),
    )(*args)
    return out.reshape(1, S, 2 * Dm)
```

```python
import functools

import jax
import jax.numpy as jnp
from jax import lax
import jax.experimental.pallas as pl
import jax.experimental.pallas.tpu as pltpu

F32 = jnp.float32
BF16 = jnp.bfloat16
U32 = jnp.uint32
LOG2E = 1.4426950408889634
NEG = -1000000000.0
LANE = 128
UA = 4
NT = (((1,), (1,)), ((), ()))


def _dot(a, b):
    return jnp.dot(a, b, preferred_element_type=F32)


def _split_jobs(raw, dst, i, rows, chunk, H, transpose=False):
    u = raw.bitcast(U32)
    pairs = H // 2

    def job(c, j):
        blk = u.at[pl.ds(pl.multiple_of((c * rows + i * chunk) * pairs, chunk * pairs), chunk * pairs)]
        w = blk[pl.ds(j, chunk, stride=pairs), :]
        if transpose:
            w = w.T
        dst(2 * j, c, pltpu.bitcast(w << 16, F32).astype(BF16))
        dst(2 * j + 1, c, pltpu.bitcast(w & jnp.uint32(0xFFFF0000), F32).astype(BF16))

    return [functools.partial(job, c, j) for c in range(raw.shape[0] // (rows * H)) for j in range(pairs)]


def _run_share(jobs, k, n):
    for job in jobs[k * len(jobs) // n:(k + 1) * len(jobs) // n]:
        job()


def _kernel(
    ax_hbm, mem_hbm, awq_hbm, awk_hbm, awv_hbm, awo_hbm,
    bx_hbm, ckv_hbm, bwq_hbm, buk_hbm, buv_hbm, bwo_hbm,
    out_hbm,
    q_all, out_v, ckv_v, bwo_v, buk_p, buv_p, sems, osems,
    *, S, Dm, H, D, M, seg, Dc,
):
    V = pltpu.VMEM
    DP = pl.cdiv(Dm, LANE) * LANE
    NP = DP // LANE
    HP = D // LANE
    CH = 64
    NC = Dc // LANE
    qscale = (D ** -0.5) * LOG2E

    def cp(src, dst, i):
        return pltpu.make_async_copy(src, dst, sems.at[i])

    def cpw(src, dst, i):
        return [cp(src.at[:, pl.ds(c * LANE, LANE)], dst.at[pl.ds(c * src.shape[0], src.shape[0])], i + c)
                for c in range(HP)]

    g3 = [cp(ckv_hbm, ckv_v, 12), cp(bwo_hbm, bwo_v, 17)]

    def phase1(wqkv, wo_p, xpad, mem_v, bxt_v, bwq_v, bwq_p, axt_v, awq_v, awk_v, awv_v, bx_v):
        g1 = [cp(bx_hbm, bxt_v, 0), *cpw(bwq_hbm, bwq_v, 1)]
        g2 = [cp(ax_hbm, axt_v, 3), cp(mem_hbm, mem_v, 4), *cpw(awq_hbm, awq_v, 5),
              *cpw(awk_hbm, awk_v, 7), *cpw(awv_hbm, awv_v, 9), *cpw(awo_hbm, wo_p, 18)]
        for c in g1:
            c.start()
        for c in g1:
            c.wait()
        for c in g2:
            c.start()
        RQ = 512

        def rows_to(ref, panel, i):
            def put(h, c, val):
                ref[panel(h, c), pl.ds(pl.multiple_of(i * CH, CH), CH), :] = val
            return put

        def wq_prep(i, carry):
            _run_share(_split_jobs(bwq_v, rows_to(bwq_p, lambda h, c: h * HP + c, i), i, Dm, CH, H), 0, 1)
            return carry

        lax.fori_loop(0, Dm // CH, wq_prep, 0)
        for r in range(S // LANE):
            bx_v[r * LANE:(r + 1) * LANE, :] = bxt_v[:, r * LANE:(r + 1) * LANE].astype(F32).T.astype(BF16)

        def q_body(h, jobs):
            w = jnp.concatenate([bwq_p[h * HP + c] for c in range(HP)], axis=1)
            for r in range(S // RQ):
                q = _dot(bx_v[r * RQ:(r + 1) * RQ, :], w)
                q_all[h, r * RQ:(r + 1) * RQ, :] = (q * qscale).astype(BF16)
                _run_share(jobs, r, S // RQ)

        na = Dm // CH
        nx = S // LANE

        def x_job(i):
            x0 = pl.multiple_of(jnp.minimum(i, nx - 1) * LANE, LANE)
            xs = axt_v[:, pl.ds(x0, LANE)].astype(F32).T
            xpad[pl.ds(x0, LANE), :] = jnp.concatenate([xs, jnp.zeros((LANE, DP - Dm), F32)], axis=1)

        def q_prep_body(i, carry):
            jobs = []
            for t, raw in enumerate((awq_v, awk_v, awv_v)):
                put = rows_to(wqkv, lambda h, c, t=t: (h * 3 + t) * HP + c, i)
                jobs += _split_jobs(raw, put, i, Dm, CH, H)
                if t < pl.cdiv(nx, na):
                    jobs.append(functools.partial(x_job, i * pl.cdiv(nx, na) + t))
            for t in range(3, pl.cdiv(nx, na)):
                jobs.append(functools.partial(x_job, i * pl.cdiv(nx, na) + t))
            q_body(H - na + i, jobs)
            return carry

        def zero_job(p):
            wqkv[jnp.minimum(p, 3 * H * HP - 1), Dm:DP, :] = jnp.zeros((DP - Dm, LANE), BF16)

        def q_zero_body(h, carry):
            nz = pl.cdiv(3 * H * HP, H - na)
            q_body(h, [functools.partial(zero_job, h * nz + p) for p in range(nz)])
            return carry

        with jax.named_scope("P1q"):
            lax.fori_loop(0, H - na, q_zero_body, 0)
        for c in g3:
            c.start()
        for c in g2:
            c.wait()
        with jax.named_scope("P1qp"):
            lax.fori_loop(0, na, q_prep_body, 0)

    def phase2(wqkv, wo_p, xpad, mem_v, buk_v, buv_v):
        g4 = [*cpw(buk_hbm, buk_v, 13), *cpw(buv_hbm, buv_v, 15)]
        for c in g4:
            c.start()
        L = M + seg
        G = 2

        def a_step(s, mem, jobs=()):
            x0 = pl.multiple_of(s * seg, seg)
            h = jnp.concatenate([mem, xpad[pl.ds(x0, seg), :]], axis=0)
            row = lax.broadcasted_iota(jnp.int32, (L, L), 0)
            col = lax.broadcasted_iota(jnp.int32, (L, L), 1)
            mask = (row < M) | (row >= col)

            def qkv(hd):
                out = []
                for t in range(3):
                    p = (hd * 3 + t) * HP
                    out.append(jnp.concatenate([_dot(h, wqkv[p + c]) for c in range(HP)], axis=1))
                q, k, v = out
                q = (q * qscale).astype(BF16).astype(F32)
                return q, k.astype(BF16), v.astype(BF16)

            def scores(qkvs):
                ps = []
                for q, k, _ in qkvs:
                    sc = lax.dot_general(q, k, NT, preferred_element_type=F32)
                    sc = jnp.where(mask, sc, NEG)
                    e = jnp.exp2(sc - jnp.max(sc, axis=1, keepdims=True))
                    p = e * (1.0 / jnp.sum(e, axis=1, keepdims=True))
                    ps.append(p.astype(BF16).astype(F32))
                return ps

            def mix(ps, qkvs):
                return [_dot(p, t[2]).astype(BF16).astype(F32) for p, t in zip(ps, qkvs)]

            acc = [None] * NP

            def outp(g, os_):
                o = jnp.concatenate(os_, axis=1)
                for c in range(NP):
                    n = min(LANE, Dm - c * LANE)
                    w = jnp.concatenate(
                        [wo_p[(kc * H + g * G + i) * Dm + c * LANE:(kc * H + g * G + i) * Dm + c * LANE + n, :]
                         for i in range(G) for kc in range(HP)], axis=1)
                    y = lax.dot_general(o, w, NT, preferred_element_type=F32)
                    acc[c] = y if acc[c] is None else acc[c] + y

            ng = H // G
            t, p, outs = {}, {}, {}
            for g in range(ng):
                t[g] = [qkv(g * G + i) for i in range(G)]
                _run_share(jobs, g, ng)
                if g >= 1:
                    p[g - 1] = scores(t[g - 1])
                if g >= 2:
                    outs[g - 2] = mix(p[g - 2], t[g - 2])
            outp(0, outs[0])
            p[ng - 1] = scores(t[ng - 1])
            outs[ng - 2] = mix(p[ng - 2], t[ng - 2])
            outp(1, outs[1])
            outp(2, outs[2])
            outs[ng - 1] = mix(p[ng - 1], t[ng - 1])
            for g in range(3, ng):
                outp(g, outs[g])
            o = jnp.concatenate(acc + [jnp.zeros((L, DP - Dm), F32)], axis=1).astype(BF16).astype(F32)
            out_v[pl.ds(x0, seg), 0:Dm] = o[M:, 0:Dm].astype(BF16)
            return o[:M, :]

        mem0 = jnp.concatenate([mem_v[...].astype(F32), jnp.zeros((M, DP - Dm), F32)], axis=1)
        ns = S // seg

        def a_prep_step(i, mem):
            def put_k(h, c, val):
                buk_p[h * HP + c, pl.ds(pl.multiple_of(i * LANE, LANE), LANE), :] = val

            def put_v(h, c, val):
                buv_p[h * NC + i, c * LANE:(c + 1) * LANE, :] = val

            jk = _split_jobs(buk_v, put_k, i, Dc, LANE, H)
            jv = _split_jobs(buv_v, put_v, i, Dc, LANE, H, transpose=True)
            return a_step(ns - NC + i, mem, [job for pair in zip(jk, jv) for job in pair])

        with jax.named_scope("P2a"):
            mem = lax.fori_loop(0, ns - NC, a_step, mem0, unroll=UA)
        for c in g4:
            c.wait()
        with jax.named_scope("P2ap"):
            lax.fori_loop(0, NC, a_prep_step, mem)

    def phase12(wqkv, wo_p, xpad, mem_v):
        pl.run_scoped(
            functools.partial(phase1, wqkv, wo_p, xpad, mem_v),
            V((Dm, S), BF16), V((HP * Dm * H, LANE), BF16), V((H * HP, Dm, LANE), BF16),
            V((Dm, S), BF16), V((HP * Dm * H, LANE), BF16), V((HP * Dm * H, LANE), BF16),
            V((HP * Dm * H, LANE), BF16), V((S, Dm), BF16))
        pl.run_scoped(
            functools.partial(phase2, wqkv, wo_p, xpad, mem_v),
            V((HP * Dc * H, LANE), BF16), V((HP * Dc * H, LANE), BF16))

    pl.run_scoped(phase12, V((3 * H * HP, DP, LANE), BF16), V((HP * H * Dm, LANE), BF16),
                  V((S, DP), F32), V((M, Dm), BF16))

    def phase3(k_v, vt_v, ctx_t):
        for c in g3:
            c.wait()
        RK = 512
        NQ = S // LANE
        NR = S // RK

        def kv_proj(h, slot, r):
            c_rows = ckv_v[r * RK:(r + 1) * RK, :]
            wk = jnp.concatenate([buk_p[h * HP + c] for c in range(HP)], axis=1)
            k_v[slot, r * RK:(r + 1) * RK, :] = _dot(c_rows, wk).astype(BF16)
            wvt = jnp.concatenate([buv_p[h * NC + c] for c in range(NC)], axis=1)
            vt_v[slot, :, r * RK:(r + 1) * RK] = lax.dot_general(
                wvt, c_rows, NT, preferred_element_type=F32).astype(BF16)

        def scores(h, slot, i):
            k0 = i * LANE
            tri = (lax.broadcasted_iota(jnp.int32, (LANE, LANE), 0)
                   <= lax.broadcasted_iota(jnp.int32, (LANE, LANE), 1))
            st = lax.dot_general(k_v[slot, 0:k0 + LANE, :], q_all[h, k0:k0 + LANE, :], NT,
                                 preferred_element_type=F32)
            sd = jnp.where(tri, st[k0:], NEG)
            st = jnp.concatenate([st[:k0], sd], axis=0) if i else sd
            return st, jnp.max(st, axis=0, keepdims=True)

        def mix(h, slot, i, st, m):
            k0 = i * LANE
            p = jnp.exp2(st - m)
            l = jnp.sum(p, axis=0, keepdims=True)
            acc = _dot(vt_v[slot, :, 0:k0 + LANE], p.astype(BF16))
            ctx_t[h, :, k0:k0 + LANE] = (acc * (1.0 / l)).astype(BF16)

        def head(h, slot, nxt):
            G = 2
            ng = NQ // G
            pend = [scores(h, slot, i) for i in range(G)]
            for g in range(ng):
                cur = pend
                if g + 1 < ng:
                    pend = [scores(h, slot, (g + 1) * G + i) for i in range(G)]
                if nxt and g >= ng - NR + 1:
                    kv_proj(h + 1, 1 - slot, g - (ng - NR + 1))
                for i in range(G):
                    mix(h, slot, g * G + i, *cur[i])
            if nxt:
                kv_proj(h + 1, 1 - slot, NR - 1)

        with jax.named_scope("P3kv0"):
            for r in range(NR):
                kv_proj(0, 0, r)

        def b_body(h, carry):
            head(h, h % 2, True)
            return carry

        with jax.named_scope("P3loop"):
            lax.fori_loop(0, H - 1, b_body, 0)
        head(H - 1, (H - 1) % 2, False)

        RO = 256
        nro = S // RO

        def ocp(r):
            return pltpu.make_async_copy(out_v.at[pl.ds(r * RO, RO)], out_hbm.at[pl.ds(r * RO, RO)],
                                         osems.at[r])

        for r in range(nro):
            ctx = jnp.concatenate([ctx_t[hh, :, r * RO:(r + 1) * RO] for hh in range(H)], axis=0)
            w = jnp.concatenate([bwo_v[hh * Dm:(hh + 1) * Dm, :] for hh in range(H)], axis=1)
            out_v[r * RO:(r + 1) * RO, Dm:2 * Dm] = _dot(w, ctx).T.astype(BF16)
            ocp(r).start()
        for r in range(nro):
            ocp(r).wait()

    pl.run_scoped(phase3, V((2, S, D), BF16), V((2, D, S), BF16), V((H, D, S), BF16))


@functools.partial(jax.jit, static_argnames=("A_seg_len",))
def pallas_concat_heads__memory_aug_recurrent_mem_tr__compressed_kv_cla__prompt_kernel(
    A_x, A_mem0, A_Wq, A_Wk, A_Wv, A_Wo, A_seg_len, B_x, B_c_kv, B_w_q, B_w_uk, B_w_uv, B_w_o,
):
    _, S, Dm = A_x.shape
    M = A_mem0.shape[1]
    _, H, D = A_Wq.shape
    Dc = B_c_kv.shape[2]
    seg = int(A_seg_len)
    args = (
        A_x.reshape(S, Dm).T, A_mem0.reshape(M, Dm),
        A_Wq.reshape(Dm * H, D), A_Wk.reshape(Dm * H, D), A_Wv.reshape(Dm * H, D),
        A_Wo.transpose(0, 2, 1).reshape(H * Dm, D),
        B_x.reshape(S, Dm).T, B_c_kv.reshape(S, Dc),
        B_w_q.reshape(Dm * H, D), B_w_uk.reshape(Dc * H, D), B_w_uv.reshape(Dc * H, D),
        B_w_o.transpose(0, 2, 1).reshape(H * Dm, D),
    )
    V = pltpu.VMEM
    scratch = [
        V((H, S, D), BF16), V((S, 2 * Dm), BF16), V((S, Dc), BF16), V((H * Dm, D), BF16),
        V((H * D // LANE, Dc, LANE), BF16), V((H * Dc // LANE, D, LANE), BF16),
        pltpu.SemaphoreType.DMA((20,)), pltpu.SemaphoreType.DMA((8,)),
    ]
    out = pl.pallas_call(
        functools.partial(_kernel, S=S, Dm=Dm, H=H, D=D, M=M, seg=seg, Dc=Dc),
        out_shape=jax.ShapeDtypeStruct((S, 2 * Dm), BF16),
        in_specs=[pl.BlockSpec(memory_space=pl.ANY)] * 12,
        out_specs=pl.BlockSpec(memory_space=pl.ANY),
        scratch_shapes=scratch,
        compiler_params=pltpu.CompilerParams(vmem_limit_bytes=120 * 2**20),
    )(*args)
    return out.reshape(1, S, 2 * Dm)
```

```python
import functools

import jax
import jax.numpy as jnp
from jax import lax
import jax.experimental.pallas as pl
import jax.experimental.pallas.tpu as pltpu

F32 = jnp.float32
BF16 = jnp.bfloat16
U32 = jnp.uint32
LOG2E = 1.4426950408889634
NEG = -1000000000.0
LANE = 128
UA = 4
NT = (((1,), (1,)), ((), ()))


def _dot(a, b):
    return jnp.dot(a, b, preferred_element_type=F32)


def _split_jobs(raw, dst, i, rows, chunk, H, transpose=False):
    u = raw.bitcast(U32)
    pairs = H // 2

    def job(c, j):
        blk = u.at[pl.ds(pl.multiple_of((c * rows + i * chunk) * pairs, chunk * pairs), chunk * pairs)]
        w = blk[pl.ds(j, chunk, stride=pairs), :]
        if transpose:
            w = w.T
        dst(2 * j, c, pltpu.bitcast(w << 16, F32).astype(BF16))
        dst(2 * j + 1, c, pltpu.bitcast(w & jnp.uint32(0xFFFF0000), F32).astype(BF16))

    return [functools.partial(job, c, j) for c in range(raw.shape[0] // (rows * H)) for j in range(pairs)]


def _run_share(jobs, k, n):
    for job in jobs[k * len(jobs) // n:(k + 1) * len(jobs) // n]:
        job()


def _kernel(
    ax_hbm, mem_hbm, awq_hbm, awk_hbm, awv_hbm, awo_hbm,
    bx_hbm, ckv_hbm, bwq_hbm, buk_hbm, buv_hbm, bwo_hbm,
    out_hbm,
    q_all, out_v, ckv_v, bwo_v, buk_p, buv_p, sems, osems,
    *, S, Dm, H, D, M, seg, Dc,
):
    V = pltpu.VMEM
    DP = pl.cdiv(Dm, LANE) * LANE
    NP = DP // LANE
    HP = D // LANE
    NC = Dc // LANE
    qscale = (D ** -0.5) * LOG2E

    def cp(src, dst, i):
        return pltpu.make_async_copy(src, dst, sems.at[i])

    def cpw(src, dst, i):
        return [cp(src.at[:, pl.ds(c * LANE, LANE)], dst.at[pl.ds(c * src.shape[0], src.shape[0])], i + c)
                for c in range(HP)]

    g3 = [cp(ckv_hbm, ckv_v, 12), cp(bwo_hbm, bwo_v, 17)]

    def phase1(wraw, wtail, wo_p, xpad, mem_v, bxt_v, bwq_v, bwq_p, axt_v, awq_v, awk_v, awv_v, bx_v):
        RQ = 512
        NRQ = S // RQ
        wq = cpw(bwq_hbm, bwq_v, 1)
        g0 = [wq[0], cp(bx_hbm.at[:, pl.ds(0, RQ)], bxt_v.at[:, pl.ds(0, RQ)], 0)]
        g1 = [cp(bx_hbm.at[:, pl.ds(RQ, S - RQ)], bxt_v.at[:, pl.ds(RQ, S - RQ)], 20), *wq[1:]]
        g2 = [cp(ax_hbm, axt_v, 3), cp(mem_hbm, mem_v, 4), *cpw(awq_hbm, awq_v, 5),
              *cpw(awk_hbm, awk_v, 7), *cpw(awv_hbm, awv_v, 9), *cpw(awo_hbm, wo_p, 18)]
        for c in g0:
            c.start()
        for c in g0:
            c.wait()
        for c in g1:
            c.start()

        def q_unit(c, r0, heads, jobs):
            for n, h in enumerate(heads):
                q = _dot(bx_v[pl.ds(r0, RQ), :], bwq_p[h * HP + c])
                q_all[h * HP + c, pl.ds(r0, RQ), :] = (q * qscale).astype(BF16)
                _run_share(jobs, n, len(heads))

        def put_q(h, c, val):
            bwq_p[h * HP + c] = val

        def bx_job(r):
            bx_v[r * LANE:(r + 1) * LANE, :] = bxt_v[:, r * LANE:(r + 1) * LANE].astype(F32).T.astype(BF16)

        wq_jobs = _split_jobs(bwq_v, put_q, 0, Dm, Dm, H)
        bx_jobs = [functools.partial(bx_job, r) for r in range(S // LANE)]
        n0 = RQ // LANE
        _run_share(bx_jobs[:n0] + wq_jobs[:1], 0, 1)
        q_unit(0, 0, range(H // 2), wq_jobs[1:H // 2])
        for c in g1:
            c.wait()
        for c in g2:
            c.start()
        q_unit(0, 0, range(H // 2, H), bx_jobs[n0:] + wq_jobs[H // 2:])

        na = 4
        CA = Dm // na
        nx = S // LANE // na
        TL = Dm - (NP - 1) * LANE

        def x_job(i):
            x0 = pl.multiple_of(i * LANE, LANE)
            xs = axt_v[:, pl.ds(x0, LANE)].astype(F32).T
            z = jnp.zeros((LANE, LANE - TL), F32)
            xpad[pl.ds(x0, LANE), :] = jnp.concatenate([xs, z, z, xs[:, Dm - TL:]], axis=1)

        def unit(u, jobs):
            q_unit(u // NRQ, pl.multiple_of((u % NRQ) * RQ, RQ), range(H), jobs)

        def plain_body(u, carry):
            unit(u, [])
            return carry

        def prep_body(i, carry):
            jobs = []
            for t, raw in enumerate((awq_v, awk_v, awv_v)):
                def put(h, c, val, t=t):
                    wraw[(h * 3 + t) * HP + c, pl.ds(pl.multiple_of(i * CA, 16), CA), :] = val
                jobs += _split_jobs(raw, put, i, Dm, CA, H)
            for k in range(nx):
                jobs.insert((k + 1) * len(jobs) // (nx + 1), functools.partial(x_job, i * nx + k))
            unit(HP * NRQ - na + i, jobs)
            return carry

        with jax.named_scope("P1q"):
            lax.fori_loop(1, HP * NRQ - na, plain_body, 0)
        for c in g3:
            c.start()
        for c in g2:
            c.wait()
        with jax.named_scope("P1qp"):
            lax.fori_loop(0, na, prep_body, 0)

        def tail_body(i, carry):
            for c in range(HP):
                wtail[i, c * TL:(c + 1) * TL, :] = wraw[i * HP + c, Dm - TL:Dm, :]
            return carry

        lax.fori_loop(0, 3 * H, tail_body, 0, unroll=8)

    def phase2(wraw, wtail, wo_p, xpad, mem_v, buk_v, buv_v):
        g4 = [*cpw(buk_hbm, buk_v, 13), *cpw(buv_hbm, buv_v, 15)]
        for c in g4:
            c.start()
        L = M + seg
        KM = (NP - 1) * LANE
        TL = Dm - KM
        GH = LANE // L
        groups = [list(range(g, min(g + GH, H))) for g in range(0, H, GH)]
        ng = len(groups)

        def a_step(s, mem, jobs=()):
            x0 = pl.multiple_of(s * seg, seg)
            xs = xpad[pl.ds(x0, seg), :]
            hm = jnp.concatenate([mem[:, :KM], xs[:, :KM]], axis=0)
            mem_hi = jnp.concatenate([mem[:, Dm:DP], mem[:, KM:Dm]], axis=1)
            ht = jnp.concatenate([mem[:, KM:DP], xs[:, KM:DP], mem_hi, xs[:, DP:]], axis=0)
            proj = {}

            def project(i0):
                ids = range(i0, i0 + 4)
                main = [[_dot(hm, wraw[i * HP + c, 0:KM, :]) for c in range(HP)] for i in ids]
                tail = _dot(ht, jnp.concatenate([wtail[i] for i in ids], axis=1))
                for n, i in enumerate(ids):
                    y = jnp.concatenate(
                        [main[n][c] + tail[c * L:(c + 1) * L, n * LANE:(n + 1) * LANE] for c in range(HP)], axis=1)
                    proj[i] = (y * qscale).astype(BF16).astype(F32) if i % 3 == 0 else y

            def stack(hs, t):
                return jnp.concatenate([proj[3 * hd + t] for hd in hs], axis=0)

            def scores(g):
                hs = groups[g]
                n = len(hs) * L
                row = lax.broadcasted_iota(jnp.int32, (n, n), 0)
                col = lax.broadcasted_iota(jnp.int32, (n, n), 1)
                sc = lax.dot_general(stack(hs, 0), stack(hs, 1).astype(BF16), NT, preferred_element_type=F32)
                out = jnp.full((n, n), -jnp.inf, F32)
                for i in range(len(hs)):
                    r, c = row - i * L, col - i * L
                    same = (r >= 0) & (r < L) & (c >= 0) & (c < L)
                    out = jnp.where(same, jnp.where((r < M) | (r >= c), sc, NEG), out)
                e = jnp.exp2(out - jnp.max(out, axis=1, keepdims=True))
                p = e * (1.0 / jnp.sum(e, axis=1, keepdims=True))
                return p.astype(BF16).astype(F32)

            o_head = {}

            def mix(g, p):
                hs = groups[g]
                o = _dot(p, stack(hs, 2).astype(BF16)).astype(BF16).astype(F32)
                for i, hd in enumerate(hs):
                    o_head[hd] = o[i * L:(i + 1) * L]

            acc = [None] * NP

            def outp(h0):
                hs = (h0, h0 + 1)
                o = jnp.concatenate([o_head[hd] for hd in hs], axis=1)
                for c in range(NP):
                    n = min(LANE, Dm - c * LANE)
                    w = jnp.concatenate(
                        [wo_p[(kc * H + hd) * Dm + c * LANE:(kc * H + hd) * Dm + c * LANE + n, :]
                         for hd in hs for kc in range(HP)], axis=1)
                    y = lax.dot_general(o, w, NT, preferred_element_type=F32)
                    acc[c] = y if acc[c] is None else acc[c] + y

            fill = [functools.partial(project, i0) for i0 in range(0, 3 * H, 4)]
            nproj = len(fill)
            fill += [functools.partial(outp, h0) for h0 in range(0, H, 2)]
            done = 0
            probs = {}
            for g in range(ng + 1):
                need = pl.cdiv(3 * (groups[min(g, ng - 1)][-1] + 1), 4) + 1
                if g >= ng - 1:
                    need = max(need, done + 1)
                while done < need:
                    fill[done]()
                    if done < nproj:
                        _run_share(jobs, done, nproj)
                    done += 1
                if g < ng:
                    probs[g] = scores(g)
                if g >= 1:
                    mix(g - 1, probs[g - 1])
            for f in fill[done:]:
                f()
            o = jnp.concatenate(acc + [jnp.zeros((L, DP - Dm), F32)], axis=1).astype(BF16).astype(F32)
            out_v[pl.ds(x0, seg), 0:Dm] = o[M:, 0:Dm].astype(BF16)
            return o[:M, :]

        mem0 = jnp.concatenate([mem_v[...].astype(F32), jnp.zeros((M, DP - Dm), F32)], axis=1)
        ns = S // seg

        def a_prep_step(i, mem):
            def put_k(h, c, val):
                buk_p[h * HP + c, pl.ds(pl.multiple_of(i * LANE, LANE), LANE), :] = val

            def put_v(h, c, val):
                buv_p[h * NC + i, c * LANE:(c + 1) * LANE, :] = val

            jk = _split_jobs(buk_v, put_k, i, Dc, LANE, H)
            jv = _split_jobs(buv_v, put_v, i, Dc, LANE, H, transpose=True)
            return a_step(ns - NC + i, mem, [job for pair in zip(jk, jv) for job in pair])

        with jax.named_scope("P2a"):
            mem = lax.fori_loop(0, ns - NC, a_step, mem0, unroll=UA)
        for c in g4:
            c.wait()
        with jax.named_scope("P2ap"):
            lax.fori_loop(0, NC, a_prep_step, mem)

    def phase12(wraw, wtail, wo_p, xpad, mem_v):
        pl.run_scoped(
            functools.partial(phase1, wraw, wtail, wo_p, xpad, mem_v),
            V((Dm, S), BF16), V((HP * Dm * H, LANE), BF16), V((H * HP, Dm, LANE), BF16),
            V((Dm, S), BF16), V((HP * Dm * H, LANE), BF16), V((HP * Dm * H, LANE), BF16),
            V((HP * Dm * H, LANE), BF16), V((S, Dm), BF16))
        pl.run_scoped(
            functools.partial(phase2, wraw, wtail, wo_p, xpad, mem_v),
            V((HP * Dc * H, LANE), BF16), V((HP * Dc * H, LANE), BF16))

    pl.run_scoped(phase12, V((3 * H * HP, Dm, LANE), BF16), V((3 * H, LANE, LANE), BF16),
                  V((HP * H * Dm, LANE), BF16), V((S, DP + LANE), F32), V((M, Dm), BF16))

    def phase3(k_v, vt_v, ctx_t):
        for c in g3:
            c.wait()
        RK = 512
        NQ = S // LANE
        NR = S // RK

        def kv_proj(h, slot, r):
            c_rows = ckv_v[r * RK:(r + 1) * RK, :]
            wk = jnp.concatenate([buk_p[h * HP + c] for c in range(HP)], axis=1)
            k_v[slot, r * RK:(r + 1) * RK, :] = _dot(c_rows, wk).astype(BF16)
            wvt = jnp.concatenate([buv_p[h * NC + c] for c in range(NC)], axis=1)
            vt_v[slot, :, r * RK:(r + 1) * RK] = lax.dot_general(
                wvt, c_rows, NT, preferred_element_type=F32).astype(BF16)

        def scores(h, slot, i):
            k0 = i * LANE
            tri = (lax.broadcasted_iota(jnp.int32, (LANE, LANE), 0)
                   <= lax.broadcasted_iota(jnp.int32, (LANE, LANE), 1))
            q = jnp.concatenate([q_all[h * HP + c, k0:k0 + LANE, :] for c in range(HP)], axis=1)
            st = lax.dot_general(k_v[slot, 0:k0 + LANE, :], q, NT, preferred_element_type=F32)
            sd = jnp.where(tri, st[k0:], NEG)
            st = jnp.concatenate([st[:k0], sd], axis=0) if i else sd
            return st, jnp.max(st, axis=0, keepdims=True)

        def mix(h, slot, i, st, m):
            k0 = i * LANE
            p = jnp.exp2(st - m)
            l = jnp.sum(p, axis=0, keepdims=True)
            acc = _dot(vt_v[slot, :, 0:k0 + LANE], p.astype(BF16))
            ctx_t[h, :, k0:k0 + LANE] = (acc * (1.0 / l)).astype(BF16)

        G = 2
        RO = G * LANE
        nro = S // RO

        def head(h, slot, fillers):
            pend = [scores(h, slot, i) for i in range(G)]
            for g in range(nro):
                cur = pend
                if g + 1 < nro:
                    pend = [scores(h, slot, (g + 1) * G + i) for i in range(G)]
                if fillers[g] is not None:
                    fillers[g]()
                for i in range(G):
                    mix(h, slot, g * G + i, *cur[i])
            fillers[nro]()

        def ocp(r):
            return pltpu.make_async_copy(out_v.at[pl.ds(r * RO, RO)], out_hbm.at[pl.ds(r * RO, RO)],
                                         osems.at[r])

        def out_proj(r):
            ctx = jnp.concatenate([ctx_t[hh, :, r * RO:(r + 1) * RO] for hh in range(H)], axis=0)
            w = jnp.concatenate([bwo_v[hh * Dm:(hh + 1) * Dm, :] for hh in range(H)], axis=1)
            out_v[r * RO:(r + 1) * RO, Dm:2 * Dm] = _dot(w, ctx).T.astype(BF16)
            ocp(r).start()

        with jax.named_scope("P3kv0"):
            for r in range(NR):
                kv_proj(0, 0, r)

        def b_body(h, carry):
            slot = h % 2
            head(h, slot, [None] * (nro + 1 - NR)
                 + [functools.partial(kv_proj, h + 1, 1 - slot, r) for r in range(NR)])
            return carry

        with jax.named_scope("P3loop"):
            lax.fori_loop(0, H - 1, b_body, 0)
        with jax.named_scope("last"):
            head(H - 1, (H - 1) % 2, [None] + [functools.partial(out_proj, r) for r in range(nro)])
            for r in range(nro):
                ocp(r).wait()

    pl.run_scoped(phase3, V((2, S, D), BF16), V((2, D, S), BF16), V((H, D, S), BF16))


@functools.partial(jax.jit, static_argnames=("A_seg_len",))
def pallas_concat_heads__memory_aug_recurrent_mem_tr__compressed_kv_cla__prompt_kernel(
    A_x, A_mem0, A_Wq, A_Wk, A_Wv, A_Wo, A_seg_len, B_x, B_c_kv, B_w_q, B_w_uk, B_w_uv, B_w_o,
):
    _, S, Dm = A_x.shape
    M = A_mem0.shape[1]
    _, H, D = A_Wq.shape
    Dc = B_c_kv.shape[2]
    seg = int(A_seg_len)
    args = (
        A_x.reshape(S, Dm).T, A_mem0.reshape(M, Dm),
        A_Wq.reshape(Dm * H, D), A_Wk.reshape(Dm * H, D), A_Wv.reshape(Dm * H, D),
        A_Wo.transpose(0, 2, 1).reshape(H * Dm, D),
        B_x.reshape(S, Dm).T, B_c_kv.reshape(S, Dc),
        B_w_q.reshape(Dm * H, D), B_w_uk.reshape(Dc * H, D), B_w_uv.reshape(Dc * H, D),
        B_w_o.transpose(0, 2, 1).reshape(H * Dm, D),
    )
    V = pltpu.VMEM
    scratch = [
        V((H * D // LANE, S, LANE), BF16), V((S, 2 * Dm), BF16), V((S, Dc), BF16), V((H * Dm, D), BF16),
        V((H * D // LANE, Dc, LANE), BF16), V((H * Dc // LANE, D, LANE), BF16),
        pltpu.SemaphoreType.DMA((21,)), pltpu.SemaphoreType.DMA((8,)),
    ]
    out = pl.pallas_call(
        functools.partial(_kernel, S=S, Dm=Dm, H=H, D=D, M=M, seg=seg, Dc=Dc),
        out_shape=jax.ShapeDtypeStruct((S, 2 * Dm), BF16),
        in_specs=[pl.BlockSpec(memory_space=pl.ANY)] * 12,
        out_specs=pl.BlockSpec(memory_space=pl.ANY),
        scratch_shapes=scratch,
        compiler_params=pltpu.CompilerParams(vmem_limit_bytes=120 * 2**20),
    )(*args)
    return out.reshape(1, S, 2 * Dm)
```

```python
import functools

import jax
import jax.numpy as jnp
from jax import lax
import jax.experimental.pallas as pl
import jax.experimental.pallas.tpu as pltpu

F32 = jnp.float32
BF16 = jnp.bfloat16
U32 = jnp.uint32
LOG2E = 1.4426950408889634
NEG = -1000000000.0
LANE = 128
UA = 4
SREF = True
RKK = 1024
FILL = '.....aAbB'
FPOS = 0
LATE = 0
DUP = False
TFIRST = False
MIXFIRST = True
OG = 2
SIZES = (3, 3, 3, 3, 3, 1)
COV = (1, 2)
LOOK = 1
NT = (((1,), (1,)), ((), ()))


def _dot(a, b):
    return jnp.dot(a, b, preferred_element_type=F32)


def _split_jobs(raw, dst, i, rows, chunk, H, transpose=False):
    u = raw.bitcast(U32)
    pairs = H // 2

    def job(c, j):
        blk = u.at[pl.ds(pl.multiple_of((c * rows + i * chunk) * pairs, chunk * pairs), chunk * pairs)]
        w = blk[pl.ds(j, chunk, stride=pairs), :]
        if transpose:
            w = w.T
        dst(2 * j, c, pltpu.bitcast(w << 16, F32).astype(BF16))
        dst(2 * j + 1, c, pltpu.bitcast(w & jnp.uint32(0xFFFF0000), F32).astype(BF16))

    return [functools.partial(job, c, j) for c in range(raw.shape[0] // (rows * H)) for j in range(pairs)]


def _run_share(jobs, k, n):
    for job in jobs[k * len(jobs) // n:(k + 1) * len(jobs) // n]:
        job()


def _kernel(
    ax_hbm, mem_hbm, awq_hbm, awk_hbm, awv_hbm, awo_hbm,
    bx_hbm, ckv_hbm, bwq_hbm, buk_hbm, buv_hbm, bwo_hbm,
    out_hbm,
    q_all, out_v, ckv_v, bwo_v, buk_p, buv_p, sems, osems,
    *, S, Dm, H, D, M, seg, Dc,
):
    V = pltpu.VMEM
    DP = pl.cdiv(Dm, LANE) * LANE
    NP = DP // LANE
    HP = D // LANE
    NC = Dc // LANE
    qscale = (D ** -0.5) * LOG2E

    def cp(src, dst, i):
        return pltpu.make_async_copy(src, dst, sems.at[i])

    def cpw(src, dst, i):
        return [cp(src.at[:, pl.ds(c * LANE, LANE)], dst.at[pl.ds(c * src.shape[0], src.shape[0])], i + c)
                for c in range(HP)]

    g3 = [cp(ckv_hbm, ckv_v, 12), cp(bwo_hbm, bwo_v, 17)]

    def phase1(wraw, wtail, wo_p, xpad, mem_v, bxt_v, bwq_v, bwq_p, axt_v, awq_v, awk_v, awv_v, bx_v):
        RQ = 512
        NRQ = S // RQ
        wq = cpw(bwq_hbm, bwq_v, 1)
        g0 = [wq[0], cp(bx_hbm.at[:, pl.ds(0, RQ)], bxt_v.at[:, pl.ds(0, RQ)], 0)]
        g1 = [cp(bx_hbm.at[:, pl.ds(RQ, S - RQ)], bxt_v.at[:, pl.ds(RQ, S - RQ)], 20), *wq[1:]]
        g2 = [cp(ax_hbm, axt_v, 3), cp(mem_hbm, mem_v, 4), *cpw(awq_hbm, awq_v, 5),
              *cpw(awk_hbm, awk_v, 7), *cpw(awv_hbm, awv_v, 9), *cpw(awo_hbm, wo_p, 18)]
        for c in g0:
            c.start()
        for c in g0:
            c.wait()
        for c in g1:
            c.start()

        def q_unit(c, r0, heads, jobs):
            for n, h in enumerate(heads):
                q = _dot(bx_v[pl.ds(r0, RQ), :], bwq_p[h * HP + c])
                q_all[h * HP + c, pl.ds(r0, RQ), :] = (q * qscale).astype(BF16)
                _run_share(jobs, n, len(heads))

        def put_q(h, c, val):
            bwq_p[h * HP + c] = val

        def bx_job(r):
            bx_v[r * LANE:(r + 1) * LANE, :] = bxt_v[:, r * LANE:(r + 1) * LANE].astype(F32).T.astype(BF16)

        wq_jobs = _split_jobs(bwq_v, put_q, 0, Dm, Dm, H)
        bx_jobs = [functools.partial(bx_job, r) for r in range(S // LANE)]
        n0 = RQ // LANE
        _run_share(bx_jobs[:n0] + wq_jobs[:1], 0, 1)
        q_unit(0, 0, range(H // 2), wq_jobs[1:H // 2])
        for c in g1:
            c.wait()
        for c in g2:
            c.start()
        q_unit(0, 0, range(H // 2, H), bx_jobs[n0:] + wq_jobs[H // 2:])

        na = 4
        CA = Dm // na
        nx = S // LANE // na
        TL = Dm - (NP - 1) * LANE

        def x_job(i):
            x0 = pl.multiple_of(i * LANE, LANE)
            xs = axt_v[:, pl.ds(x0, LANE)].astype(F32).T
            z = jnp.zeros((LANE, LANE - TL), F32)
            xpad[pl.ds(x0, LANE), :] = jnp.concatenate([xs, z, z, xs[:, Dm - TL:]], axis=1)

        def unit(u, jobs):
            q_unit(u // NRQ, pl.multiple_of((u % NRQ) * RQ, RQ), range(H), jobs)

        def plain_body(u, carry):
            unit(u, [])
            return carry

        def prep_body(i, carry):
            jobs = []
            for t, raw in enumerate((awq_v, awk_v, awv_v)):
                def put(h, c, val, t=t):
                    wraw[(h * 3 + t) * HP + c, pl.ds(pl.multiple_of(i * CA, 16), CA), :] = val
                jobs += _split_jobs(raw, put, i, Dm, CA, H)
            for k in range(nx):
                jobs.insert((k + 1) * len(jobs) // (nx + 1), functools.partial(x_job, i * nx + k))
            unit(HP * NRQ - na + i, jobs)
            return carry

        with jax.named_scope("P1q"):
            lax.fori_loop(1, HP * NRQ - na, plain_body, 0)
        for c in g3:
            c.start()
        for c in g2:
            c.wait()
        with jax.named_scope("P1qp"):
            lax.fori_loop(0, na, prep_body, 0)

        def tail_body(i, carry):
            for c in range(HP):
                wtail[i, c * TL:(c + 1) * TL, :] = wraw[i * HP + c, Dm - TL:Dm, :]
            return carry

        lax.fori_loop(0, 3 * H, tail_body, 0, unroll=8)

    def phase2(wraw, wtail, wo_p, xpad, mem_v, buk_v, buv_v):
        g4 = [*cpw(buk_hbm, buk_v, 13), *cpw(buv_hbm, buv_v, 15)]
        for c in g4:
            c.start()
        L = M + seg
        KM = (NP - 1) * LANE
        TL = Dm - KM
        GH = LANE // L
        groups = [list(range(sum(SIZES[:g]), sum(SIZES[:g + 1]))) for g in range(len(SIZES))]
        ng = len(groups)

        def a_step(s, mem, jobs=()):
            x0 = pl.multiple_of(s * seg, seg)
            xs = xpad[pl.ds(x0, seg), :]
            hm = jnp.concatenate([mem[:, :KM], xs[:, :KM]], axis=0)
            low = lax.broadcasted_iota(jnp.int32, (M, LANE), 1) < TL
            if DUP:
                ht = jnp.concatenate([jnp.where(low, mem[:, KM:], 0.0), xs[:, KM:DP],
                                      jnp.where(low, 0.0, mem[:, KM:]), xs[:, DP:]], axis=0)
            else:
                mem_hi = jnp.concatenate([mem[:, Dm:DP], mem[:, KM:Dm]], axis=1)
                ht = jnp.concatenate([mem[:, KM:DP], xs[:, KM:DP], mem_hi, xs[:, DP:]], axis=0)
            proj = {}

            def project(i0):
                ids = range(i0, i0 + 4)
                if TFIRST and i0:
                    tail = _dot(ht, jnp.concatenate([wtail[i] for i in ids], axis=1))
                main = [[_dot(hm, wraw[i * HP + c, 0:KM, :]) for c in range(HP)] for i in ids]
                if not (TFIRST and i0):
                    tail = _dot(ht, jnp.concatenate([wtail[i] for i in ids], axis=1))
                for n, i in enumerate(ids):
                    y = jnp.concatenate(
                        [main[n][c] + tail[c * L:(c + 1) * L, n * LANE:(n + 1) * LANE] for c in range(HP)], axis=1)
                    proj[i] = (y * qscale).astype(BF16).astype(F32) if i % 3 == 0 else y

            def stack(hs, t):
                return jnp.concatenate([proj[3 * hd + t] for hd in hs], axis=0)

            def scores(g):
                hs = groups[g]
                n = len(hs) * L
                row = lax.broadcasted_iota(jnp.int32, (n, n), 0)
                col = lax.broadcasted_iota(jnp.int32, (n, n), 1)
                sc = lax.dot_general(stack(hs, 0), stack(hs, 1).astype(BF16), NT, preferred_element_type=F32)
                out = jnp.full((n, n), -jnp.inf, F32)
                for i in range(len(hs)):
                    r, c = row - i * L, col - i * L
                    same = (r >= 0) & (r < L) & (c >= 0) & (c < L)
                    out = jnp.where(same, jnp.where((r < M) | (r >= c), sc, NEG), out)
                e = jnp.exp2(out - jnp.max(out, axis=1, keepdims=True))
                p = e * (1.0 / jnp.sum(e, axis=1, keepdims=True))
                return p.astype(BF16).astype(F32)

            o_head = {}

            def mix(g, p):
                hs = groups[g]
                o = _dot(p, stack(hs, 2).astype(BF16)).astype(BF16).astype(F32)
                for i, hd in enumerate(hs):
                    o_head[hd] = o[i * L:(i + 1) * L]

            acc = [None] * NP

            def outp(h0, cols):
                hs = range(h0, h0 + OG)
                o = jnp.concatenate([o_head[hd] for hd in hs], axis=1)
                for c in cols:
                    n = min(LANE, Dm - c * LANE)
                    w = jnp.concatenate(
                        [wo_p[(kc * H + hd) * Dm + c * LANE:(kc * H + hd) * Dm + c * LANE + n, :]
                         for hd in hs for kc in range(HP)], axis=1)
                    y = lax.dot_general(o, jnp.concatenate([w] * (LANE // n if DUP else 1), axis=0), NT,
                                        preferred_element_type=F32)
                    acc[c] = y if acc[c] is None else acc[c] + y

            fill = [functools.partial(project, i0) for i0 in range(0, 3 * H, 4)]
            nproj = len(fill)
            late = H - LATE
            fill += [functools.partial(outp, h0, range(NP if h0 < late else NP - 1)) for h0 in range(0, H, OG)]
            fill += [functools.partial(outp, h0, [NP - 1]) for h0 in range(late, H, OG)]
            done = 0
            probs = {}
            for g in range(ng + 1):
                need = pl.cdiv(3 * (groups[min(g, ng - 1)][-1] + 1), 4) + LOOK
                if g >= ng - 1:
                    need = max(need, done + COV[g - ng + 1])
                while done < need:
                    fill[done]()
                    if done < nproj:
                        _run_share(jobs, done, nproj)
                    done += 1
                if g >= 1 and MIXFIRST:
                    mix(g - 1, probs[g - 1])
                if g < ng:
                    probs[g] = scores(g)
                if g >= 1 and not MIXFIRST:
                    mix(g - 1, probs[g - 1])
            for f in fill[done:]:
                f()
            o = jnp.concatenate(acc + ([] if DUP else [jnp.zeros((L, DP - Dm), F32)]), axis=1).astype(BF16).astype(F32)
            out_v[pl.ds(x0, seg), 0:Dm] = o[M:, 0:Dm].astype(BF16)
            return o[:M, :]

        mem0 = mem_v[...].astype(F32)
        mem0 = jnp.concatenate([mem0, mem0[:, KM:]], axis=1)
        ns = S // seg

        def a_prep_step(i, mem):
            def put_k(h, c, val):
                buk_p[h * HP + c, pl.ds(pl.multiple_of(i * LANE, LANE), LANE), :] = val

            def put_v(h, c, val):
                buv_p[h * NC + i, c * LANE:(c + 1) * LANE, :] = val

            jk = _split_jobs(buk_v, put_k, i, Dc, LANE, H)
            jv = _split_jobs(buv_v, put_v, i, Dc, LANE, H, transpose=True)
            return a_step(ns - NC + i, mem, [job for pair in zip(jk, jv) for job in pair])

        with jax.named_scope("P2a"):
            mem = lax.fori_loop(0, ns - NC, a_step, mem0, unroll=UA)
        for c in g4:
            c.wait()
        with jax.named_scope("P2ap"):
            lax.fori_loop(0, NC, a_prep_step, mem)

    def phase12(wraw, wtail, wo_p, xpad, mem_v):
        pl.run_scoped(
            functools.partial(phase1, wraw, wtail, wo_p, xpad, mem_v),
            V((Dm, S), BF16), V((HP * Dm * H, LANE), BF16), V((H * HP, Dm, LANE), BF16),
            V((Dm, S), BF16), V((HP * Dm * H, LANE), BF16), V((HP * Dm * H, LANE), BF16),
            V((HP * Dm * H, LANE), BF16), V((S, Dm), BF16))
        pl.run_scoped(
            functools.partial(phase2, wraw, wtail, wo_p, xpad, mem_v),
            V((HP * Dc * H, LANE), BF16), V((HP * Dc * H, LANE), BF16))

    pl.run_scoped(phase12, V((3 * H * HP, Dm, LANE), BF16), V((3 * H, LANE, LANE), BF16),
                  V((HP * H * Dm, LANE), BF16), V((S, DP + LANE), F32), V((M, Dm), BF16))

    def phase3(k_v, vt_v, ctx_t, s_v):
        for c in g3:
            c.wait()
        RK = RKK
        NQ = S // LANE
        NR = S // RK

        def kv_proj(h, slot, r, which="kv"):
            c_rows = ckv_v[r * RK:(r + 1) * RK, :]
            if "k" in which:
                wk = jnp.concatenate([buk_p[h * HP + c] for c in range(HP)], axis=1)
                k_v[slot, r * RK:(r + 1) * RK, :] = _dot(c_rows, wk).astype(BF16)
            if "v" in which:
                wvt = jnp.concatenate([buv_p[h * NC + c] for c in range(NC)], axis=1)
                vt_v[slot, :, r * RK:(r + 1) * RK] = lax.dot_general(
                    wvt, c_rows, NT, preferred_element_type=F32).astype(BF16)

        def fold(x, op):
            x = x.reshape(LANE // 8, 8, LANE)
            return op(x, axis=0)

        def scores(h, slot, i):
            k0 = i * LANE
            tri = (lax.broadcasted_iota(jnp.int32, (LANE, LANE), 0)
                   <= lax.broadcasted_iota(jnp.int32, (LANE, LANE), 1))
            q = jnp.concatenate([q_all[h * HP + c, k0:k0 + LANE, :] for c in range(HP)], axis=1)
            st = lax.dot_general(k_v[slot, 0:k0 + LANE, :], q, NT, preferred_element_type=F32)
            m = None
            blks = []
            for c in range(i + 1):
                blk = st[c * LANE:(c + 1) * LANE]
                if c == i:
                    blk = jnp.where(tri, blk, NEG)
                if SREF:
                    s_v[i % 4, c * LANE:(c + 1) * LANE, :] = blk
                blks.append(blk)
                pm = fold(blk, jnp.max)
                m = pm if m is None else jnp.maximum(m, pm)
            return blks, jnp.max(m, axis=0, keepdims=True)

        def mix(h, slot, i, blks, m):
            k0 = i * LANE
            l = None
            ps = []
            for c in range(i + 1):
                blk = s_v[i % 4, c * LANE:(c + 1) * LANE, :] if SREF else blks[c]
                p = jnp.exp2(blk - m)
                pl_ = fold(p, jnp.sum)
                l = pl_ if l is None else l + pl_
                ps.append(p.astype(BF16))
            l = jnp.sum(l, axis=0, keepdims=True)
            acc = _dot(vt_v[slot, :, 0:k0 + LANE], jnp.concatenate(ps, axis=0))
            ctx_t[h, :, k0:k0 + LANE] = (acc * (1.0 / l)).astype(BF16)

        G = 2
        RO = G * LANE
        nro = S // RO

        def head(h, slot, fillers):
            pend = [scores(h, slot, i) for i in range(G)]
            for g in range(nro):
                cur = pend
                if fillers[g] is not None and FPOS == 1:
                    fillers[g]()
                if g + 1 < nro:
                    pend = [scores(h, slot, (g + 1) * G + i) for i in range(G)]
                if fillers[g] is not None and FPOS == 0:
                    fillers[g]()
                for i in range(G):
                    mix(h, slot, g * G + i, *cur[i])
                    if fillers[g] is not None and FPOS == 2 and i == 0:
                        fillers[g]()
            fillers[nro]()

        def ocp(r):
            return pltpu.make_async_copy(out_v.at[pl.ds(r * RO, RO)], out_hbm.at[pl.ds(r * RO, RO)],
                                         osems.at[r])

        def out_proj(r):
            ctx = jnp.concatenate([ctx_t[hh, :, r * RO:(r + 1) * RO] for hh in range(H)], axis=0)
            w = jnp.concatenate([bwo_v[hh * Dm:(hh + 1) * Dm, :] for hh in range(H)], axis=1)
            out_v[r * RO:(r + 1) * RO, Dm:2 * Dm] = _dot(w, ctx).T.astype(BF16)
            ocp(r).start()

        with jax.named_scope("P3kv0"):
            for r in range(NR):
                kv_proj(0, 0, r)

        def b_body(h, carry):
            slot = h % 2
            fill = []
            for ch in FILL:
                if ch == '.':
                    fill.append(None)
                elif ch.isdigit():
                    fill.append(functools.partial(kv_proj, h + 1, 1 - slot, int(ch)))
                elif ch.islower():
                    fill.append(functools.partial(kv_proj, h + 1, 1 - slot, ord(ch) - ord('a'), "k"))
                else:
                    fill.append(functools.partial(kv_proj, h + 1, 1 - slot, ord(ch) - ord('A'), "v"))
            head(h, slot, fill)
            return carry

        with jax.named_scope("P3loop"):
            lax.fori_loop(0, H - 1, b_body, 0)
        with jax.named_scope("last"):
            head(H - 1, (H - 1) % 2, [None] + [functools.partial(out_proj, r) for r in range(nro)])
            for r in range(nro):
                ocp(r).wait()

    pl.run_scoped(phase3, V((2, S, D), BF16), V((2, D, S), BF16), V((H, D, S), BF16), V((4, S, LANE), F32))


@functools.partial(jax.jit, static_argnames=("A_seg_len",))
def pallas_concat_heads__memory_aug_recurrent_mem_tr__compressed_kv_cla__prompt_kernel(
    A_x, A_mem0, A_Wq, A_Wk, A_Wv, A_Wo, A_seg_len, B_x, B_c_kv, B_w_q, B_w_uk, B_w_uv, B_w_o,
):
    _, S, Dm = A_x.shape
    M = A_mem0.shape[1]
    _, H, D = A_Wq.shape
    Dc = B_c_kv.shape[2]
    seg = int(A_seg_len)
    args = (
        A_x.reshape(S, Dm).T, A_mem0.reshape(M, Dm),
        A_Wq.reshape(Dm * H, D), A_Wk.reshape(Dm * H, D), A_Wv.reshape(Dm * H, D),
        A_Wo.transpose(0, 2, 1).reshape(H * Dm, D),
        B_x.reshape(S, Dm).T, B_c_kv.reshape(S, Dc),
        B_w_q.reshape(Dm * H, D), B_w_uk.reshape(Dc * H, D), B_w_uv.reshape(Dc * H, D),
        B_w_o.transpose(0, 2, 1).reshape(H * Dm, D),
    )
    V = pltpu.VMEM
    scratch = [
        V((H * D // LANE, S, LANE), BF16), V((S, 2 * Dm), BF16), V((S, Dc), BF16), V((H * Dm, D), BF16),
        V((H * D // LANE, Dc, LANE), BF16), V((H * Dc // LANE, D, LANE), BF16),
        pltpu.SemaphoreType.DMA((21,)), pltpu.SemaphoreType.DMA((8,)),
    ]
    out = pl.pallas_call(
        functools.partial(_kernel, S=S, Dm=Dm, H=H, D=D, M=M, seg=seg, Dc=Dc),
        out_shape=jax.ShapeDtypeStruct((S, 2 * Dm), BF16),
        in_specs=[pl.BlockSpec(memory_space=pl.ANY)] * 12,
        out_specs=pl.BlockSpec(memory_space=pl.ANY),
        scratch_shapes=scratch,
        compiler_params=pltpu.CompilerParams(vmem_limit_bytes=120 * 2**20),
    )(*args)
    return out.reshape(1, S, 2 * Dm)
```

```python
import functools

import jax
import jax.numpy as jnp
from jax import lax
import jax.experimental.pallas as pl
import jax.experimental.pallas.tpu as pltpu

F32 = jnp.float32
BF16 = jnp.bfloat16
U32 = jnp.uint32
LOG2E = 1.4426950408889634
NEG = -1000000000.0
LANE = 128
UA = 4
SREF = True
RKK = 1024
FILL = '.....aAbB'
FPOS = 0
LATE = 0
DUP = False
TFIRST = False
MIXFIRST = True
OG = 2
SIZES = (3, 3, 3, 3, 3, 1)
COV = (1, 2)
LOOK = 1
NT = (((1,), (1,)), ((), ()))


def _dot(a, b):
    return jnp.dot(a, b, preferred_element_type=F32)


def _split_jobs(raw, dst, i, rows, chunk, H, transpose=False):
    u = raw.bitcast(U32)
    pairs = H // 2

    def job(c, j):
        blk = u.at[pl.ds(pl.multiple_of((c * rows + i * chunk) * pairs, chunk * pairs), chunk * pairs)]
        w = blk[pl.ds(j, chunk, stride=pairs), :]
        if transpose:
            w = w.T
        dst(2 * j, c, pltpu.bitcast(w << 16, F32).astype(BF16))
        dst(2 * j + 1, c, pltpu.bitcast(w & jnp.uint32(0xFFFF0000), F32).astype(BF16))

    return [functools.partial(job, c, j) for c in range(raw.shape[0] // (rows * H)) for j in range(pairs)]


def _run_share(jobs, k, n):
    for job in jobs[k * len(jobs) // n:(k + 1) * len(jobs) // n]:
        job()


def _kernel(
    ax_hbm, mem_hbm, awq_hbm, awk_hbm, awv_hbm, awo_hbm,
    bx_hbm, ckv_hbm, bwq_hbm, buk_hbm, buv_hbm, bwo_hbm,
    out_hbm,
    q_all, out_v, ckv_v, bwo_v, buk_p, buv_p, sems, osems,
    *, S, Dm, H, D, M, seg, Dc,
):
    V = pltpu.VMEM
    DP = pl.cdiv(Dm, LANE) * LANE
    NP = DP // LANE
    HP = D // LANE
    NC = Dc // LANE
    qscale = (D ** -0.5) * LOG2E

    def cp(src, dst, i):
        return pltpu.make_async_copy(src, dst, sems.at[i])

    def cpw(src, dst, i):
        return [cp(src.at[:, pl.ds(c * LANE, LANE)], dst.at[pl.ds(c * src.shape[0], src.shape[0])], i + c)
                for c in range(HP)]

    g3 = [cp(ckv_hbm, ckv_v, 12), cp(bwo_hbm, bwo_v, 17)]

    def phase1(wraw, wtail, wo_p, xpad, mem_v, bxt_v, bwq_v, bwq_p, axt_v, awq_v, awk_v, awv_v, bx_v):
        RQ = 512
        NRQ = S // RQ
        wq = cpw(bwq_hbm, bwq_v, 1)
        g0 = [wq[0], cp(bx_hbm.at[:, pl.ds(0, RQ)], bxt_v.at[:, pl.ds(0, RQ)], 0)]
        g1 = [cp(bx_hbm.at[:, pl.ds(RQ, S - RQ)], bxt_v.at[:, pl.ds(RQ, S - RQ)], 20), *wq[1:]]
        g2 = [cp(ax_hbm, axt_v, 3), *cpw(awq_hbm, awq_v, 5), *cpw(awk_hbm, awk_v, 7), *cpw(awv_hbm, awv_v, 9)]
        g2b = [cp(mem_hbm, mem_v, 4), *cpw(awo_hbm, wo_p, 18)]
        for c in g0:
            c.start()
        for c in g0:
            c.wait()
        for c in g1:
            c.start()

        def q_unit(c, r0, heads, jobs):
            for n, h in enumerate(heads):
                q = _dot(bx_v[pl.ds(r0, RQ), :], bwq_p[h * HP + c])
                q_all[h * HP + c, pl.ds(r0, RQ), :] = (q * qscale).astype(BF16)
                _run_share(jobs, n, len(heads))

        def put_q(h, c, val):
            bwq_p[h * HP + c] = val

        def bx_job(r):
            bx_v[r * LANE:(r + 1) * LANE, :] = bxt_v[:, r * LANE:(r + 1) * LANE].astype(F32).T.astype(BF16)

        wq_jobs = _split_jobs(bwq_v, put_q, 0, Dm, Dm, H)
        bx_jobs = [functools.partial(bx_job, r) for r in range(S // LANE)]
        n0 = RQ // LANE
        _run_share(bx_jobs[:n0] + wq_jobs[:1], 0, 1)
        q_unit(0, 0, range(H // 2), wq_jobs[1:H // 2])
        for c in g1:
            c.wait()
        for c in g2:
            c.start()
        q_unit(0, 0, range(H // 2, H), bx_jobs[n0:] + wq_jobs[H // 2:])

        na = 4
        CA = Dm // na
        nx = S // LANE // na
        TL = Dm - (NP - 1) * LANE

        def x_job(i):
            x0 = pl.multiple_of(i * LANE, LANE)
            xs = axt_v[:, pl.ds(x0, LANE)].astype(F32).T
            z = jnp.zeros((LANE, LANE - TL), F32)
            xpad[pl.ds(x0, LANE), :] = jnp.concatenate([xs, z, z, xs[:, Dm - TL:]], axis=1)

        def unit(u, jobs):
            q_unit(u // NRQ, pl.multiple_of((u % NRQ) * RQ, RQ), range(H), jobs)

        def plain_body(u, carry):
            unit(u, [])
            return carry

        def prep_body(i, carry):
            jobs = []
            for t, raw in enumerate((awq_v, awk_v, awv_v)):
                def put(h, c, val, t=t):
                    wraw[(h * 3 + t) * HP + c, pl.ds(pl.multiple_of(i * CA, 16), CA), :] = val
                jobs += _split_jobs(raw, put, i, Dm, CA, H)
            for k in range(nx):
                jobs.insert((k + 1) * len(jobs) // (nx + 1), functools.partial(x_job, i * nx + k))
            unit(HP * NRQ - na + i, jobs)
            return carry

        with jax.named_scope("P1q"):
            lax.fori_loop(1, HP * NRQ - na, plain_body, 0)
        for c in g2:
            c.wait()
        for c in g2b:
            c.start()
        for c in g3:
            c.start()
        with jax.named_scope("P1qp"):
            lax.fori_loop(0, na, prep_body, 0)

        def tail_body(i, carry):
            for c in range(HP):
                wtail[i, c * TL:(c + 1) * TL, :] = wraw[i * HP + c, Dm - TL:Dm, :]
            return carry

        lax.fori_loop(0, 3 * H, tail_body, 0, unroll=8)
        for c in g2b:
            c.wait()

    def phase2(wraw, wtail, wo_p, xpad, mem_v, buk_v, buv_v):
        g4 = [*cpw(buk_hbm, buk_v, 13), *cpw(buv_hbm, buv_v, 15)]
        for c in g4:
            c.start()
        L = M + seg
        KM = (NP - 1) * LANE
        TL = Dm - KM
        GH = LANE // L
        groups = [list(range(sum(SIZES[:g]), sum(SIZES[:g + 1]))) for g in range(len(SIZES))]
        ng = len(groups)

        def a_step(s, mem, jobs=()):
            x0 = pl.multiple_of(s * seg, seg)
            xs = xpad[pl.ds(x0, seg), :]
            hm = jnp.concatenate([mem[:, :KM], xs[:, :KM]], axis=0)
            low = lax.broadcasted_iota(jnp.int32, (M, LANE), 1) < TL
            if DUP:
                ht = jnp.concatenate([jnp.where(low, mem[:, KM:], 0.0), xs[:, KM:DP],
                                      jnp.where(low, 0.0, mem[:, KM:]), xs[:, DP:]], axis=0)
            else:
                mem_hi = jnp.concatenate([mem[:, Dm:DP], mem[:, KM:Dm]], axis=1)
                ht = jnp.concatenate([mem[:, KM:DP], xs[:, KM:DP], mem_hi, xs[:, DP:]], axis=0)
            proj = {}

            def project(i0):
                ids = range(i0, i0 + 4)
                if TFIRST and i0:
                    tail = _dot(ht, jnp.concatenate([wtail[i] for i in ids], axis=1))
                main = [[_dot(hm, wraw[i * HP + c, 0:KM, :]) for c in range(HP)] for i in ids]
                if not (TFIRST and i0):
                    tail = _dot(ht, jnp.concatenate([wtail[i] for i in ids], axis=1))
                for n, i in enumerate(ids):
                    y = jnp.concatenate(
                        [main[n][c] + tail[c * L:(c + 1) * L, n * LANE:(n + 1) * LANE] for c in range(HP)], axis=1)
                    proj[i] = (y * qscale).astype(BF16).astype(F32) if i % 3 == 0 else y

            def stack(hs, t):
                return jnp.concatenate([proj[3 * hd + t] for hd in hs], axis=0)

            def scores(g):
                hs = groups[g]
                n = len(hs) * L
                row = lax.broadcasted_iota(jnp.int32, (n, n), 0)
                col = lax.broadcasted_iota(jnp.int32, (n, n), 1)
                sc = lax.dot_general(stack(hs, 0), stack(hs, 1).astype(BF16), NT, preferred_element_type=F32)
                out = jnp.full((n, n), -jnp.inf, F32)
                for i in range(len(hs)):
                    r, c = row - i * L, col - i * L
                    same = (r >= 0) & (r < L) & (c >= 0) & (c < L)
                    out = jnp.where(same, jnp.where((r < M) | (r >= c), sc, NEG), out)
                e = jnp.exp2(out - jnp.max(out, axis=1, keepdims=True))
                p = e * (1.0 / jnp.sum(e, axis=1, keepdims=True))
                return p.astype(BF16).astype(F32)

            o_head = {}

            def mix(g, p):
                hs = groups[g]
                o = _dot(p, stack(hs, 2).astype(BF16)).astype(BF16).astype(F32)
                for i, hd in enumerate(hs):
                    o_head[hd] = o[i * L:(i + 1) * L]

            acc = [None] * NP

            def outp(h0, cols):
                hs = range(h0, h0 + OG)
                o = jnp.concatenate([o_head[hd] for hd in hs], axis=1)
                for c in cols:
                    n = min(LANE, Dm - c * LANE)
                    w = jnp.concatenate(
                        [wo_p[(kc * H + hd) * Dm + c * LANE:(kc * H + hd) * Dm + c * LANE + n, :]
                         for hd in hs for kc in range(HP)], axis=1)
                    y = lax.dot_general(o, jnp.concatenate([w] * (LANE // n if DUP else 1), axis=0), NT,
                                        preferred_element_type=F32)
                    acc[c] = y if acc[c] is None else acc[c] + y

            fill = [functools.partial(project, i0) for i0 in range(0, 3 * H, 4)]
            nproj = len(fill)
            late = H - LATE
            fill += [functools.partial(outp, h0, range(NP if h0 < late else NP - 1)) for h0 in range(0, H, OG)]
            fill += [functools.partial(outp, h0, [NP - 1]) for h0 in range(late, H, OG)]
            done = 0
            probs = {}
            for g in range(ng + 1):
                need = pl.cdiv(3 * (groups[min(g, ng - 1)][-1] + 1), 4) + LOOK
                if g >= ng - 1:
                    need = max(need, done + COV[g - ng + 1])
                while done < need:
                    fill[done]()
                    if done < nproj:
                        _run_share(jobs, done, nproj)
                    done += 1
                if g >= 1 and MIXFIRST:
                    mix(g - 1, probs[g - 1])
                if g < ng:
                    probs[g] = scores(g)
                if g >= 1 and not MIXFIRST:
                    mix(g - 1, probs[g - 1])
            for f in fill[done:]:
                f()
            o = jnp.concatenate(acc + ([] if DUP else [jnp.zeros((L, DP - Dm), F32)]), axis=1).astype(BF16).astype(F32)
            out_v[pl.ds(x0, seg), 0:Dm] = o[M:, 0:Dm].astype(BF16)
            return o[:M, :]

        mem0 = mem_v[...].astype(F32)
        mem0 = jnp.concatenate([mem0, jnp.zeros((M, DP - Dm), F32)], axis=1)
        ns = S // seg

        def a_prep_step(i, mem):
            def put_k(h, c, val):
                buk_p[h * HP + c, pl.ds(pl.multiple_of(i * LANE, LANE), LANE), :] = val

            def put_v(h, c, val):
                buv_p[h * NC + i, c * LANE:(c + 1) * LANE, :] = val

            jk = _split_jobs(buk_v, put_k, i, Dc, LANE, H)
            jv = _split_jobs(buv_v, put_v, i, Dc, LANE, H, transpose=True)
            return a_step(ns - NC + i, mem, [job for pair in zip(jk, jv) for job in pair])

        with jax.named_scope("P2a"):
            mem = lax.fori_loop(0, ns - NC, a_step, mem0, unroll=UA)
        for c in g4:
            c.wait()
        with jax.named_scope("P2ap"):
            lax.fori_loop(0, NC, a_prep_step, mem)

    def phase12(wraw, wtail, wo_p, xpad, mem_v):
        pl.run_scoped(
            functools.partial(phase1, wraw, wtail, wo_p, xpad, mem_v),
            V((Dm, S), BF16), V((HP * Dm * H, LANE), BF16), V((H * HP, Dm, LANE), BF16),
            V((Dm, S), BF16), V((HP * Dm * H, LANE), BF16), V((HP * Dm * H, LANE), BF16),
            V((HP * Dm * H, LANE), BF16), V((S, Dm), BF16))
        pl.run_scoped(
            functools.partial(phase2, wraw, wtail, wo_p, xpad, mem_v),
            V((HP * Dc * H, LANE), BF16), V((HP * Dc * H, LANE), BF16))

    pl.run_scoped(phase12, V((3 * H * HP, Dm, LANE), BF16), V((3 * H, LANE, LANE), BF16),
                  V((HP * H * Dm, LANE), BF16), V((S, DP + LANE), F32), V((M, Dm), BF16))

    def phase3(k_v, vt_v, ctx_t, s_v):
        for c in g3:
            c.wait()
        RK = RKK
        NQ = S // LANE
        NR = S // RK

        def kv_proj(h, slot, r, which="kv"):
            c_rows = ckv_v[r * RK:(r + 1) * RK, :]
            if "k" in which:
                wk = jnp.concatenate([buk_p[h * HP + c] for c in range(HP)], axis=1)
                k_v[slot, r * RK:(r + 1) * RK, :] = _dot(c_rows, wk).astype(BF16)
            if "v" in which:
                wvt = jnp.concatenate([buv_p[h * NC + c] for c in range(NC)], axis=1)
                vt_v[slot, :, r * RK:(r + 1) * RK] = lax.dot_general(
                    wvt, c_rows, NT, preferred_element_type=F32).astype(BF16)

        def fold(x, op):
            x = x.reshape(LANE // 8, 8, LANE)
            return op(x, axis=0)

        def scores(h, slot, i):
            k0 = i * LANE
            tri = (lax.broadcasted_iota(jnp.int32, (LANE, LANE), 0)
                   <= lax.broadcasted_iota(jnp.int32, (LANE, LANE), 1))
            q = jnp.concatenate([q_all[h * HP + c, k0:k0 + LANE, :] for c in range(HP)], axis=1)
            st = lax.dot_general(k_v[slot, 0:k0 + LANE, :], q, NT, preferred_element_type=F32)
            m = None
            blks = []
            for c in range(i + 1):
                blk = st[c * LANE:(c + 1) * LANE]
                if c == i:
                    blk = jnp.where(tri, blk, NEG)
                if SREF:
                    s_v[i % 4, c * LANE:(c + 1) * LANE, :] = blk
                blks.append(blk)
                pm = fold(blk, jnp.max)
                m = pm if m is None else jnp.maximum(m, pm)
            return blks, jnp.max(m, axis=0, keepdims=True)

        def mix(h, slot, i, blks, m):
            k0 = i * LANE
            l = None
            ps = []
            for c in range(i + 1):
                blk = s_v[i % 4, c * LANE:(c + 1) * LANE, :] if SREF else blks[c]
                p = jnp.exp2(blk - m)
                pl_ = fold(p, jnp.sum)
                l = pl_ if l is None else l + pl_
                ps.append(p.astype(BF16))
            l = jnp.sum(l, axis=0, keepdims=True)
            acc = _dot(vt_v[slot, :, 0:k0 + LANE], jnp.concatenate(ps, axis=0))
            ctx_t[h, :, k0:k0 + LANE] = (acc * (1.0 / l)).astype(BF16)

        G = 2
        RO = G * LANE
        nro = S // RO

        def head(h, slot, fillers):
            pend = [scores(h, slot, i) for i in range(G)]
            for g in range(nro):
                cur = pend
                if fillers[g] is not None and FPOS == 1:
                    fillers[g]()
                if g + 1 < nro:
                    pend = [scores(h, slot, (g + 1) * G + i) for i in range(G)]
                if fillers[g] is not None and FPOS == 0:
                    fillers[g]()
                for i in range(G):
                    mix(h, slot, g * G + i, *cur[i])
                    if fillers[g] is not None and FPOS == 2 and i == 0:
                        fillers[g]()
            fillers[nro]()

        def ocp(r):
            return pltpu.make_async_copy(out_v.at[pl.ds(r * RO, RO)], out_hbm.at[pl.ds(r * RO, RO)],
                                         osems.at[r])

        def out_proj(r):
            ctx = jnp.concatenate([ctx_t[hh, :, r * RO:(r + 1) * RO] for hh in range(H)], axis=0)
            w = jnp.concatenate([bwo_v[hh * Dm:(hh + 1) * Dm, :] for hh in range(H)], axis=1)
            out_v[r * RO:(r + 1) * RO, Dm:2 * Dm] = _dot(w, ctx).T.astype(BF16)
            ocp(r).start()

        with jax.named_scope("P3kv0"):
            for r in range(NR):
                kv_proj(0, 0, r)

        def b_body(h, carry):
            slot = h % 2
            fill = []
            for ch in FILL:
                if ch == '.':
                    fill.append(None)
                elif ch.isdigit():
                    fill.append(functools.partial(kv_proj, h + 1, 1 - slot, int(ch)))
                elif ch.islower():
                    fill.append(functools.partial(kv_proj, h + 1, 1 - slot, ord(ch) - ord('a'), "k"))
                else:
                    fill.append(functools.partial(kv_proj, h + 1, 1 - slot, ord(ch) - ord('A'), "v"))
            head(h, slot, fill)
            return carry

        with jax.named_scope("P3loop"):
            lax.fori_loop(0, H - 1, b_body, 0)
        with jax.named_scope("last"):
            head(H - 1, (H - 1) % 2, [None] + [functools.partial(out_proj, r) for r in range(nro)])
            for r in range(nro):
                ocp(r).wait()

    pl.run_scoped(phase3, V((2, S, D), BF16), V((2, D, S), BF16), V((H, D, S), BF16), V((4, S, LANE), F32))


@functools.partial(jax.jit, static_argnames=("A_seg_len",))
def pallas_concat_heads__memory_aug_recurrent_mem_tr__compressed_kv_cla__prompt_kernel(
    A_x, A_mem0, A_Wq, A_Wk, A_Wv, A_Wo, A_seg_len, B_x, B_c_kv, B_w_q, B_w_uk, B_w_uv, B_w_o,
):
    _, S, Dm = A_x.shape
    M = A_mem0.shape[1]
    _, H, D = A_Wq.shape
    Dc = B_c_kv.shape[2]
    seg = int(A_seg_len)
    args = (
        A_x.reshape(S, Dm).T, A_mem0.reshape(M, Dm),
        A_Wq.reshape(Dm * H, D), A_Wk.reshape(Dm * H, D), A_Wv.reshape(Dm * H, D),
        A_Wo.transpose(0, 2, 1).reshape(H * Dm, D),
        B_x.reshape(S, Dm).T, B_c_kv.reshape(S, Dc),
        B_w_q.reshape(Dm * H, D), B_w_uk.reshape(Dc * H, D), B_w_uv.reshape(Dc * H, D),
        B_w_o.transpose(0, 2, 1).reshape(H * Dm, D),
    )
    V = pltpu.VMEM
    scratch = [
        V((H * D // LANE, S, LANE), BF16), V((S, 2 * Dm), BF16), V((S, Dc), BF16), V((H * Dm, D), BF16),
        V((H * D // LANE, Dc, LANE), BF16), V((H * Dc // LANE, D, LANE), BF16),
        pltpu.SemaphoreType.DMA((21,)), pltpu.SemaphoreType.DMA((8,)),
    ]
    out = pl.pallas_call(
        functools.partial(_kernel, S=S, Dm=Dm, H=H, D=D, M=M, seg=seg, Dc=Dc),
        out_shape=jax.ShapeDtypeStruct((S, 2 * Dm), BF16),
        in_specs=[pl.BlockSpec(memory_space=pl.ANY)] * 12,
        out_specs=pl.BlockSpec(memory_space=pl.ANY),
        scratch_shapes=scratch,
        compiler_params=pltpu.CompilerParams(vmem_limit_bytes=120 * 2**20),
    )(*args)
    return out.reshape(1, S, 2 * Dm)
```

```python
import functools

import jax
import jax.numpy as jnp
from jax import lax
import jax.experimental.pallas as pl
import jax.experimental.pallas.tpu as pltpu

F32 = jnp.float32
BF16 = jnp.bfloat16
U32 = jnp.uint32
LOG2E = 1.4426950408889634
NEG = -1000000000.0 * LOG2E
LANE = 128
NT = (((1,), (1,)), ((), ()))


def _dot(a, b):
    return jnp.dot(a, b, preferred_element_type=F32)


def _dot_nt(a, b):
    return lax.dot_general(a, b, NT, preferred_element_type=F32)


def _split_jobs(raw, dst, i, rows, chunk, H, transpose=False):
    u = raw.bitcast(U32)
    pairs = H // 2

    def job(c, j):
        blk = u.at[pl.ds(pl.multiple_of((c * rows + i * chunk) * pairs, chunk * pairs), chunk * pairs)]
        w = blk[pl.ds(j, chunk, stride=pairs), :]
        if transpose:
            w = w.T
        dst(2 * j, c, pltpu.bitcast(w << 16, F32).astype(BF16))
        dst(2 * j + 1, c, pltpu.bitcast(w & jnp.uint32(0xFFFF0000), F32).astype(BF16))

    return [functools.partial(job, c, j) for c in range(raw.shape[0] // (rows * H)) for j in range(pairs)]


def _run_share(jobs, k, n):
    for job in jobs[k * len(jobs) // n:(k + 1) * len(jobs) // n]:
        job()


def _start(copies):
    for c in copies:
        c.start()


def _wait(copies):
    for c in copies:
        c.wait()


def _kernel(
    ax_hbm, mem_hbm, awq_hbm, awk_hbm, awv_hbm, awo_hbm,
    bx_hbm, ckv_hbm, bwq_hbm, buk_hbm, buv_hbm, bwo_hbm,
    out_hbm,
    q_all, out_v, ckv_v, bwo_v, buk_p, buv_p, sems, osems,
    *, S, Dm, H, D, M, seg, Dc,
):
    V = pltpu.VMEM
    NP = pl.cdiv(Dm, LANE)
    DP = NP * LANE
    KM = (NP - 1) * LANE
    TL = Dm - KM
    HP = D // LANE
    NC = Dc // LANE
    assert HP == 2 and HP * TL == LANE
    L = M + seg
    NS = S // seg
    RQ = 512
    NRQ = S // RQ
    ND = 2
    NA = 2
    qscale = (D ** -0.5) * LOG2E

    def cp(src, dst, i):
        return pltpu.make_async_copy(src, dst, sems.at[i])

    def cpw(src, dst, i):
        n = src.shape[0]
        return [cp(src.at[:, pl.ds(c * LANE, LANE)], dst.at[pl.ds(c * n, n)], i + c) for c in range(HP)]

    g3 = [cp(ckv_hbm, ckv_v, 12), cp(bwo_hbm, bwo_v, 17)]

    def q_proj(bx_v, bwq_p, panel, r0, n):
        q = _dot(bx_v[pl.ds(r0, n), :], bwq_p[panel])
        q_all[panel, pl.ds(r0, n), :] = (q * qscale).astype(BF16)

    def phase1(wmain, wtail, wo_p, xpad, mem_v, bx_v, bwq_p,
               bxt0_v, bxt1_v, bwq0_v, bwq1_v, axt_v, awq_v, awk_v, awv_v):
        g0 = [cp(bwq_hbm.at[:, pl.ds(0, LANE)], bwq0_v, 1), cp(bx_hbm.at[:, pl.ds(0, RQ)], bxt0_v, 0)]
        g1 = [cp(bx_hbm.at[:, pl.ds(RQ, S - RQ)], bxt1_v, 20), cp(bwq_hbm.at[:, pl.ds(LANE, LANE)], bwq1_v, 2)]
        g2 = [cp(ax_hbm, axt_v, 3), *cpw(awq_hbm, awq_v, 5), *cpw(awk_hbm, awk_v, 7), *cpw(awv_hbm, awv_v, 9)]
        g2b = [cp(mem_hbm, mem_v, 4), *cpw(awo_hbm, wo_p, 18)]
        _start(g0)
        _wait(g0)
        _start(g1)

        def q_unit(c, r0, heads, jobs):
            for n, h in enumerate(heads):
                q_proj(bx_v, bwq_p, h * HP + c, r0, RQ)
                _run_share(jobs, n, len(heads))

        def put_q(c0, h, c, val):
            bwq_p[h * HP + c0 + c] = val

        n0 = RQ // LANE

        def bx_job(r):
            src, k = (bxt0_v, r) if r < n0 else (bxt1_v, r - n0)
            bx_v[r * LANE:(r + 1) * LANE, :] = src[:, k * LANE:(k + 1) * LANE].astype(F32).T.astype(BF16)

        wq_jobs = [job for c, raw in enumerate((bwq0_v, bwq1_v))
                   for job in _split_jobs(raw, functools.partial(put_q, c), 0, Dm, Dm, H)]
        bx_jobs = [functools.partial(bx_job, r) for r in range(S // LANE)]
        _run_share(bx_jobs[:n0] + wq_jobs[:1], 0, 1)
        q_unit(0, 0, range(H // 2), wq_jobs[1:H // 2])
        _wait(g1)
        _start(g2)
        q_unit(0, 0, range(H // 2, H), bx_jobs[n0:] + wq_jobs[H // 2:])

        CA = Dm // NA
        nx = S // LANE // NA
        first_prep = HP * NRQ - ND - NA

        def x_job(i):
            x0 = pl.multiple_of(i * LANE, LANE)
            xs = axt_v[:, pl.ds(x0, LANE)].astype(F32).T
            z = jnp.zeros((LANE, LANE - TL), F32)
            xpad[pl.ds(x0, LANE), :] = jnp.concatenate([xs, z, z, xs[:, KM:]], axis=1)

        def unit(u, jobs):
            q_unit(u // NRQ, pl.multiple_of((u % NRQ) * RQ, RQ), range(H), jobs)

        def plain_body(u, carry):
            unit(u, [])
            return carry

        def prep_body(i, carry):
            jobs = []
            for t, raw in enumerate((awq_v, awk_v, awv_v)):
                def put(h, c, val, t=t):
                    wmain[(h * 3 + t) * HP + c, pl.ds(pl.multiple_of(i * CA, 16), CA), :] = val
                jobs += _split_jobs(raw, put, i, Dm, CA, H)
            for k in range(nx):
                jobs.insert((k + 1) * len(jobs) // (nx + 1), functools.partial(x_job, i * nx + k))
            unit(first_prep + i, jobs)
            return carry

        lax.fori_loop(1, first_prep, plain_body, 0)
        _wait(g2)
        _start(g2b)
        _start(g3)
        lax.fori_loop(0, NA, prep_body, 0)

        def tail_body(i, carry):
            for c in range(HP):
                wtail[i, c * TL:(c + 1) * TL, :] = wmain[i * HP + c, KM:Dm, :]
            return carry

        lax.fori_loop(0, 3 * H, tail_body, 0, unroll=8)
        _wait(g2b)

    def phase2(wmain, wtail, wo_p, xpad, mem_v, bx_v, bwq_p, buk_v, buv_v):
        g4 = [*cpw(buk_hbm, buk_v, 13), *cpw(buv_hbm, buv_v, 15)]
        _start(g4)
        GH = LANE // L
        groups = [list(range(g, min(g + GH, H))) for g in range(0, H, GH)]
        ng = len(groups)

        def a_step(s, mem, jobs=()):
            x0 = pl.multiple_of(s * seg, seg)
            xs = xpad[pl.ds(x0, seg), :]
            hm = jnp.concatenate([mem[:, :KM], xs[:, :KM]], axis=0)
            mem_hi = jnp.concatenate([mem[:, Dm:DP], mem[:, KM:Dm]], axis=1)
            ht = jnp.concatenate([mem[:, KM:DP], xs[:, KM:DP], mem_hi, xs[:, DP:]], axis=0)
            proj = {}

            def project(i0):
                ids = range(i0, i0 + 4)
                main = [[_dot(hm, wmain[i * HP + c, 0:KM, :]) for c in range(HP)] for i in ids]
                tail = _dot(ht, jnp.concatenate([wtail[i] for i in ids], axis=1))
                for n, i in enumerate(ids):
                    y = jnp.concatenate(
                        [main[n][c] + tail[c * L:(c + 1) * L, n * LANE:(n + 1) * LANE] for c in range(HP)], axis=1)
                    proj[i] = (y * qscale).astype(BF16).astype(F32) if i % 3 == 0 else y

            def stack(hs, t):
                return jnp.concatenate([proj[3 * hd + t] for hd in hs], axis=0)

            def scores(g):
                hs = groups[g]
                n = len(hs) * L
                row = lax.broadcasted_iota(jnp.int32, (n, n), 0)
                col = lax.broadcasted_iota(jnp.int32, (n, n), 1)
                sc = _dot_nt(stack(hs, 0), stack(hs, 1).astype(BF16))
                out = jnp.full((n, n), -jnp.inf, F32)
                for i in range(len(hs)):
                    r, c = row - i * L, col - i * L
                    same = (r >= 0) & (r < L) & (c >= 0) & (c < L)
                    out = jnp.where(same, jnp.where((r < M) | (r >= c), sc, NEG), out)
                e = jnp.exp2(out - jnp.max(out, axis=1, keepdims=True))
                p = e * (1.0 / jnp.sum(e, axis=1, keepdims=True))
                return p.astype(BF16).astype(F32)

            o_head = {}

            def mix(g, p):
                hs = groups[g]
                o = _dot(p, stack(hs, 2).astype(BF16)).astype(BF16).astype(F32)
                for i, hd in enumerate(hs):
                    o_head[hd] = o[i * L:(i + 1) * L]

            acc = [None] * NP

            def out_proj(h0):
                hs = (h0, h0 + 1)
                o = jnp.concatenate([o_head[hd] for hd in hs], axis=1)
                for c in range(NP):
                    n = min(LANE, Dm - c * LANE)
                    w = jnp.concatenate(
                        [wo_p[(kc * H + hd) * Dm + c * LANE:(kc * H + hd) * Dm + c * LANE + n, :]
                         for hd in hs for kc in range(HP)], axis=1)
                    y = _dot_nt(o, w)
                    acc[c] = y if acc[c] is None else acc[c] + y

            fill = [functools.partial(project, i0) for i0 in range(0, 3 * H, 4)]
            nproj = len(fill)
            fill += [functools.partial(out_proj, h0) for h0 in range(0, H, 2)]
            done = 0
            probs = {}
            for g in range(ng + 1):
                need = pl.cdiv(3 * (groups[min(g, ng - 1)][-1] + 1), 4) + 1
                if g >= ng - 1:
                    need = max(need, done + g - ng + 2)
                while done < need:
                    fill[done]()
                    if done < nproj:
                        _run_share(jobs, done, nproj)
                    done += 1
                if g >= 1:
                    mix(g - 1, probs[g - 1])
                if g < ng:
                    probs[g] = scores(g)
            for f in fill[done:]:
                f()
            per = NS // H
            n = ND * RQ // per
            q_proj(bx_v, bwq_p, (s // per) * HP + HP - 1, pl.multiple_of(S - ND * RQ + (s % per) * n, n), n)
            o = jnp.concatenate(acc + [jnp.zeros((L, DP - Dm), F32)], axis=1).astype(BF16).astype(F32)
            out_v[pl.ds(x0, seg), 0:Dm] = o[M:, 0:Dm].astype(BF16)
            return o[:M, :]

        def a_prep_step(i, mem):
            def put_k(h, c, val):
                buk_p[h * HP + c, pl.ds(pl.multiple_of(i * LANE, LANE), LANE), :] = val

            def put_v(h, c, val):
                buv_p[h * NC + i, c * LANE:(c + 1) * LANE, :] = val

            jk = _split_jobs(buk_v, put_k, i, Dc, LANE, H)
            jv = _split_jobs(buv_v, put_v, i, Dc, LANE, H, transpose=True)
            return a_step(NS - NC + i, mem, [job for pair in zip(jk, jv) for job in pair])

        mem = jnp.concatenate([mem_v[...].astype(F32), jnp.zeros((M, DP - Dm), F32)], axis=1)
        mem = lax.fori_loop(0, NS - NC, a_step, mem, unroll=4)
        _wait(g4)
        lax.fori_loop(0, NC, a_prep_step, mem)

    def phase12(*refs):
        pl.run_scoped(
            functools.partial(phase1, *refs),
            V((Dm, RQ), BF16), V((Dm, S - RQ), BF16), V((Dm * H, LANE), BF16), V((Dm * H, LANE), BF16),
            V((Dm, S), BF16), V((HP * Dm * H, LANE), BF16), V((HP * Dm * H, LANE), BF16),
            V((HP * Dm * H, LANE), BF16))
        pl.run_scoped(
            functools.partial(phase2, *refs),
            V((HP * Dc * H, LANE), BF16), V((HP * Dc * H, LANE), BF16))

    pl.run_scoped(phase12, V((3 * H * HP, Dm, LANE), BF16), V((3 * H, LANE, LANE), BF16),
                  V((HP * H * Dm, LANE), BF16), V((S, DP + LANE), F32), V((M, Dm), BF16),
                  V((S, Dm), BF16), V((H * HP, Dm, LANE), BF16))

    def phase3(k_v, vt_v, ctx_t, s_v):
        RK = 1024
        NR = S // RK
        G = 2
        RO = G * LANE
        nro = S // RO

        def kv_proj(h, slot, r, which):
            rows = pl.ds(r * RK, RK)
            c_rows = ckv_v[rows, :]
            if "k" in which:
                wk = jnp.concatenate([buk_p[h * HP + c] for c in range(HP)], axis=1)
                k_v[slot, rows, :] = _dot(c_rows, wk).astype(BF16)
            if "v" in which:
                wvt = jnp.concatenate([buv_p[h * NC + c] for c in range(NC)], axis=1)
                vt_v[slot, :, rows] = _dot_nt(wvt, c_rows).astype(BF16)

        def fold(x, op):
            return op(x.reshape(LANE // 8, 8, LANE), axis=0)

        def scores(h, slot, i):
            k0 = i * LANE
            tri = (lax.broadcasted_iota(jnp.int32, (LANE, LANE), 0)
                   <= lax.broadcasted_iota(jnp.int32, (LANE, LANE), 1))
            q = jnp.concatenate([q_all[h * HP + c, k0:k0 + LANE, :] for c in range(HP)], axis=1)
            st = _dot_nt(k_v[slot, 0:k0 + LANE, :], q)
            m = None
            for c in range(i + 1):
                blk = st[c * LANE:(c + 1) * LANE]
                if c == i:
                    blk = jnp.where(tri, blk, NEG)
                s_v[i % (2 * G), c * LANE:(c + 1) * LANE, :] = blk
                pm = fold(blk, jnp.max)
                m = pm if m is None else jnp.maximum(m, pm)
            return jnp.max(m, axis=0, keepdims=True)

        def mix(h, slot, i, m):
            k0 = i * LANE
            l = None
            ps = []
            for c in range(i + 1):
                p = jnp.exp2(s_v[i % (2 * G), c * LANE:(c + 1) * LANE, :] - m)
                ps_ = fold(p, jnp.sum)
                l = ps_ if l is None else l + ps_
                ps.append(p.astype(BF16))
            l = jnp.sum(l, axis=0, keepdims=True)
            acc = _dot(vt_v[slot, :, 0:k0 + LANE], jnp.concatenate(ps, axis=0))
            ctx_t[h, :, k0:k0 + LANE] = (acc * (1.0 / l)).astype(BF16)

        def head(h, slot, fillers):
            pend = [scores(h, slot, i) for i in range(G)]
            for g in range(nro):
                cur = pend
                if g + 1 < nro:
                    pend = [scores(h, slot, (g + 1) * G + i) for i in range(G)]
                if fillers[g] is not None:
                    fillers[g]()
                for i in range(G):
                    mix(h, slot, g * G + i, cur[i])
            fillers[nro]()

        def ocp(r):
            return pltpu.make_async_copy(out_v.at[pl.ds(r * RO, RO)], out_hbm.at[pl.ds(r * RO, RO)],
                                         osems.at[r])

        def out_proj(r):
            ctx = jnp.concatenate([ctx_t[hh, :, r * RO:(r + 1) * RO] for hh in range(H)], axis=0)
            w = jnp.concatenate([bwo_v[hh * Dm:(hh + 1) * Dm, :] for hh in range(H)], axis=1)
            out_v[r * RO:(r + 1) * RO, Dm:2 * Dm] = _dot(w, ctx).T.astype(BF16)
            ocp(r).start()

        _wait(g3)
        for r in range(NR):
            kv_proj(0, 0, r, "kv")

        def b_body(h, carry):
            slot = h % 2
            head(h, slot, [None] * (nro + 1 - 2 * NR)
                 + [functools.partial(kv_proj, h + 1, 1 - slot, r, which) for r in range(NR) for which in "kv"])
            return carry

        lax.fori_loop(0, H - 1, b_body, 0)
        head(H - 1, (H - 1) % 2, [None] + [functools.partial(out_proj, r) for r in range(nro)])
        for r in range(nro):
            ocp(r).wait()

    pl.run_scoped(phase3, V((2, S, D), BF16), V((2, D, S), BF16), V((H, D, S), BF16), V((4, S, LANE), F32))


@functools.partial(jax.jit, static_argnames=("A_seg_len",))
def pallas_concat_heads__memory_aug_recurrent_mem_tr__compressed_kv_cla__prompt_kernel(
    A_x, A_mem0, A_Wq, A_Wk, A_Wv, A_Wo, A_seg_len, B_x, B_c_kv, B_w_q, B_w_uk, B_w_uv, B_w_o,
):
    _, S, Dm = A_x.shape
    M = A_mem0.shape[1]
    _, H, D = A_Wq.shape
    Dc = B_c_kv.shape[2]
    assert B_x.shape == A_x.shape and B_c_kv.shape[1] == S and B_w_q.shape == A_Wq.shape
    args = (
        A_x.reshape(S, Dm).T, A_mem0.reshape(M, Dm),
        A_Wq.reshape(Dm * H, D), A_Wk.reshape(Dm * H, D), A_Wv.reshape(Dm * H, D),
        A_Wo.transpose(0, 2, 1).reshape(H * Dm, D),
        B_x.reshape(S, Dm).T, B_c_kv.reshape(S, Dc),
        B_w_q.reshape(Dm * H, D), B_w_uk.reshape(Dc * H, D), B_w_uv.reshape(Dc * H, D),
        B_w_o.transpose(0, 2, 1).reshape(H * Dm, D),
    )
    V = pltpu.VMEM
    scratch = [
        V((H * D // LANE, S, LANE), BF16), V((S, 2 * Dm), BF16), V((S, Dc), BF16), V((H * Dm, D), BF16),
        V((H * D // LANE, Dc, LANE), BF16), V((H * Dc // LANE, D, LANE), BF16),
        pltpu.SemaphoreType.DMA((21,)), pltpu.SemaphoreType.DMA((S // (2 * LANE),)),
    ]
    out = pl.pallas_call(
        functools.partial(_kernel, S=S, Dm=Dm, H=H, D=D, M=M, seg=int(A_seg_len), Dc=Dc),
        out_shape=jax.ShapeDtypeStruct((S, 2 * Dm), BF16),
        in_specs=[pl.BlockSpec(memory_space=pl.ANY)] * 12,
        out_specs=pl.BlockSpec(memory_space=pl.ANY),
        scratch_shapes=scratch,
        compiler_params=pltpu.CompilerParams(vmem_limit_bytes=120 * 2**20),
    )(*args)
    return out.reshape(1, S, 2 * Dm)
```
